```python
import jax
import jax.numpy as jnp

def _softmax(x, axis=-1):
    return jax.nn.softmax(x, axis=axis)

def _gelu(x):
    return jax.nn.gelu(x, approximate=True)

def _silu(x):
    return jax.nn.silu(x)

def _sigmoid(x):
    return jax.nn.sigmoid(x)

def _layernorm(x, axis=-1, eps=1e-05):
    m = jnp.mean(x, axis=axis, keepdims=True)
    v = jnp.var(x, axis=axis, keepdims=True)
    return (x - m) / jnp.sqrt(v + eps)

def _scatter_add(tgt, idx, src, axis=0):
    return tgt.at[idx].add(src)

def _segment_sum(src, seg, n):
    return jax.ops.segment_sum(src, seg, n)

class _Rng:

    def __init__(self, key):
        self._k = key

    def _next(self):
        self._k, sub = jax.random.split(self._k)
        return sub

    def normal(self, shape):
        return jax.random.normal(self._next(), shape, dtype=jnp.bfloat16)

    def randint(self, lo, hi, shape):
        return jax.random.randint(self._next(), shape, lo, hi, dtype=jnp.int32)

    def uniform(self, shape, lo=0.0, hi=1.0):
        return jax.random.uniform(self._next(), shape, jnp.bfloat16, lo, hi)

    def permutation(self, n):
        return jax.random.permutation(self._next(), n)
kernel_name = 'gated_mix__memory_aug_recurrent_mem_tr__ssm_conv_h3__prompt'

def setup_inputs():
    _rng = _Rng(jax.random.key(int.from_bytes(__import__("os").urandom(4), "little")))
    _w = lambda a: (lambda t: t.astype(jnp.bfloat16) if jnp.issubdtype(t.dtype, jnp.floating) else t)(jnp.asarray(a))

    def _A_setup():
        B, S, Dm = (1, 2048, 640)
        H, Dh = (32, 192)
        M, seg = (8, 32)
        seg = min(seg, S)
        S = S // seg * seg
        return {'x': _w((lambda *s: _rng.normal(s) * 0.05)(B, S, Dm)), 'mem0': _w((lambda *s: _rng.normal(s) * 0.05)(B, M, Dm)), 'Wq': _w((lambda *s: _rng.normal(s) * 0.05)(Dm, H, Dh) * Dm ** (-0.5)), 'Wk': _w((lambda *s: _rng.normal(s) * 0.05)(Dm, H, Dh) * Dm ** (-0.5)), 'Wv': _w((lambda *s: _rng.normal(s) * 0.05)(Dm, H, Dh) * Dm ** (-0.5)), 'Wo': _w((lambda *s: _rng.normal(s) * 0.05)(H, Dh, Dm) * (H * Dh) ** (-0.5)), 'seg_len': seg}
    _A_in = _A_setup()

    def _B_setup():
        B, S, D = (1, 2048, 640)
        ks = 4
        return {'q': _w((lambda *s: _rng.normal(s) * 0.05)(B, S, D)), 'k': _w((lambda *s: _rng.normal(s) * 0.05)(B, S, D)), 'v': _w((lambda *s: _rng.normal(s) * 0.05)(B, S, D)), 'shift_k': _w((lambda *s: _rng.normal(s) * 0.05)(D, ks) * 0.5), 'ssm_k': _w((lambda *s: _rng.normal(s) * 0.05)(D, S) * (1.0 / S ** 0.5)), 'ssm_D': _w((lambda *s: _rng.normal(s) * 0.05)(D))}
    _B_in = _B_setup()
    return {'A_x': _A_in['x'], 'A_mem0': _A_in['mem0'], 'A_Wq': _A_in['Wq'], 'A_Wk': _A_in['Wk'], 'A_Wv': _A_in['Wv'], 'A_Wo': _A_in['Wo'], 'A_seg_len': _A_in['seg_len'], 'B_q': _B_in['q'], 'B_k': _B_in['k'], 'B_v': _B_in['v'], 'B_shift_k': _B_in['shift_k'], 'B_ssm_k': _B_in['ssm_k'], 'B_ssm_D': _B_in['ssm_D'], 'gate_w': _w((lambda *s: _rng.normal(s) * 0.05)(640))}

def reference(A_x, A_mem0, A_Wq, A_Wk, A_Wv, A_Wo, A_seg_len, B_q, B_k, B_v, B_shift_k, B_ssm_k, B_ssm_D, gate_w):

    def _A_ref(x, mem0, Wq, Wk, Wv, Wo, seg_len):
        B, S, Dm = x.shape
        H, Dh = (Wq.shape[1], Wq.shape[2])
        M = mem0.shape[1]
        scale = Dh ** (-0.5)
        n_seg = S // seg_len
        L = M + seg_len
        idx = jnp.arange(L)
        mask = (idx[:, None] < M) | (idx[:, None] >= idx[None, :])
        mem = mem0
        outs = []
        for s in range(n_seg):
            xs = x[:, s * seg_len:(s + 1) * seg_len, :].copy()
            h = jnp.concatenate([mem, xs], axis=1)
            q = jnp.einsum('btd,dhe->bhte', h, Wq)
            k = jnp.einsum('btd,dhe->bhte', h, Wk)
            v = jnp.einsum('btd,dhe->bhte', h, Wv)
            scores = jnp.einsum('bhqe,bhke->bhqk', q, k) * scale
            scores = jnp.where(mask[None, None], scores, -1000000000.0)
            p = _softmax(scores, axis=-1)
            o = jnp.einsum('bhqk,bhke->bhqe', p, v)
            o = jnp.einsum('bhte,hed->btd', o, Wo)
            mem = o[:, :M, :].copy()
            outs.append(o[:, M:, :])
        return jnp.concatenate(outs, axis=1)

    def _B_ref(q, k, v, shift_k, ssm_k, ssm_D):
        B, S, D = q.shape
        ks = shift_k.shape[-1]
        k_pad = jnp.pad(k, ((0, 0), (ks - 1, 0), (0, 0)))
        k_shift = jnp.zeros_like(k)
        for t in range(ks):
            k_shift = k_shift + k_pad[:, t:t + S, :] * shift_k[:, ks - 1 - t][None, None, :]
        kv = k_shift * v
        L = 2 * S
        kv_pad = jnp.pad(kv, ((0, 0), (0, S), (0, 0)))
        kf_pad = jnp.pad(ssm_k, ((0, 0), (0, S)))
        kv_f = (lambda x, axes=(-2, -1): jnp.fft.rfft2(x.astype(jnp.float32), axes=axes))(kv_pad[:, None, :, :], axes=(1, 2))
        kf_f = (lambda x, axes=(-2, -1): jnp.fft.rfft2(x.astype(jnp.float32), axes=axes))(kf_pad[:, None, :], axes=(1, 2))
        kf_f = (lambda x, *d: x.transpose(*d))(kf_f, 1, 2, 0)
        y_f = kv_f * kf_f[None, :, :, :]
        y = (lambda x, s, axes=(-2, -1): jnp.fft.irfft2(x, s=s, axes=axes).astype(jnp.bfloat16))(y_f, (1, L), axes=(1, 2))[:, 0, :S, :]
        y = y + kv * ssm_D[None, None, :]
        return q * y
    x = A_x
    g = _sigmoid((x * gate_w).sum(-1, keepdims=True))
    a = _A_ref(x, A_mem0, A_Wq, A_Wk, A_Wv, A_Wo, A_seg_len)
    b = _B_ref(x, B_k, B_v, B_shift_k, B_ssm_k, B_ssm_D)
    return g * a + (1 - g) * b
```

```python
import numpy as np

import jax
import jax.numpy as jnp
import jax.experimental.pallas as pl
import jax.experimental.pallas.tpu as pltpu

_BLK = 128


def _dft_matrices():
    f = np.concatenate([np.arange(0, _BLK, 2), np.arange(1, _BLK, 2)])
    t = np.arange(_BLK)
    ang = 2.0 * np.pi * (f[:, None] + 0.5) * t[None, :] / (2 * _BLK)
    fwd = np.concatenate([np.cos(ang), -np.sin(ang)], axis=0)
    inv = fwd.T / _BLK
    return fwd.astype(np.float32), inv.astype(np.float32)


def _dot(a, b):
    return jax.lax.dot_general(
        a, b, (((1,), (0,)), ((), ())), preferred_element_type=jnp.float32)


def _dot_nt(a, b):
    return jax.lax.dot_general(
        a, b, (((1,), (1,)), ((), ())), preferred_element_type=jnp.float32)


def _make_kernel(S, D, H, Dh, M, seg, ks):
    L = M + seg
    n_seg = S // seg
    n_pair = H // 2
    PW = 2 * Dh
    n_blk = S // _BLK
    n_ct = D // 128
    scale = float(Dh) ** -0.5
    out_chunk = 8
    f32, bf16 = jnp.float32, jnp.bfloat16

    def kernel(x_hbm, mem0_ref, wq_hbm, wk_hbm, wv_hbm, wo_hbm, k_hbm, v_hbm,
               shift_ref, g_hbm, dskip_ref, gw_ref, fwd_ref, inv_ref,
               out_hbm,
               x_vm, k_vm, v_vm, g_vm, stage, wqkv, wo_vm,
               kpad, u_hat, g_hat, y_hat, kv_vm, b_vm, gate_vm, out_vm,
               in_sem, w_sem, wo_sem, out_sem):
        in_copies = [
            pltpu.make_async_copy(x_hbm, x_vm, in_sem.at[0]),
            pltpu.make_async_copy(k_hbm, k_vm, in_sem.at[1]),
            pltpu.make_async_copy(v_hbm, v_vm, in_sem.at[2]),
            pltpu.make_async_copy(g_hbm, g_vm, in_sem.at[3]),
        ]
        for c in in_copies:
            c.start()

        def w_copy(m, j):
            src = (wq_hbm, wk_hbm, wv_hbm)[m]
            return pltpu.make_async_copy(
                src.at[pl.ds(j * PW, PW), :], stage.at[j, m], w_sem.at[j * 3 + m])

        for j in range(n_pair):
            for m in range(3):
                w_copy(m, j).start()
        wo_copy = pltpu.make_async_copy(wo_hbm, wo_vm, wo_sem)
        wo_copy.start()
        for c in in_copies:
            c.wait()

        gw = gw_ref[...].astype(f32)

        def gate_body(i, carry):
            rows = pl.ds(pl.multiple_of(i * 128, 128), 128)
            z = jnp.sum(x_vm[rows, :].astype(f32) * gw, axis=-1, keepdims=True)
            gate_vm[rows, :] = jnp.broadcast_to(jax.nn.sigmoid(z), (128, 128))
            return carry

        jax.lax.fori_loop(0, S // 128, gate_body, 0)

        kpad[0:8, :] = jnp.zeros((8, 128), f32)
        half = _BLK // 2

        def b_tile(c, carry):
            c0 = pl.multiple_of(c * 128, 128)
            cols = pl.ds(c0, 128)
            kpad[8:8 + S, :] = k_vm[:, cols].astype(f32)
            sh = shift_ref[:, cols].astype(f32)
            fwd = fwd_ref[...]
            for a in range(n_blk):
                acc = kpad[pl.ds(8 + a * _BLK, _BLK), :] * sh[0:1, :]
                for i in range(1, ks):
                    acc = acc + kpad[pl.ds(8 + a * _BLK - i, _BLK), :] * sh[i:i + 1, :]
                kv = (acc * v_vm[pl.ds(a * _BLK, _BLK), cols].astype(f32)).astype(bf16)
                kv_vm[pl.ds(a * _BLK, _BLK), :] = kv
                u_hat[a] = _dot(fwd, kv)
            prev = None
            for a in range(n_blk):
                cur = _dot_nt(fwd, g_vm[cols, pl.ds(a * _BLK, _BLK)])
                if prev is None:
                    g_hat[a] = cur
                else:
                    g_hat[a, 0:half, :] = cur[0:half] - prev[_BLK:_BLK + half]
                    g_hat[a, half:_BLK, :] = cur[half:_BLK] + prev[_BLK + half:]
                    g_hat[a, _BLK:_BLK + half, :] = cur[_BLK:_BLK + half] + prev[0:half]
                    g_hat[a, _BLK + half:, :] = cur[_BLK + half:] - prev[half:_BLK]
                prev = cur

            def freq_body(r, carry2):
                re = pl.ds(pl.multiple_of(r * 8, 8), 8)
                im = pl.ds(pl.multiple_of(_BLK + r * 8, 8), 8)
                ur = [u_hat[a, re, :] for a in range(n_blk)]
                ui = [u_hat[a, im, :] for a in range(n_blk)]
                for a in range(n_blk):
                    yr = yi = None
                    for j in range(a + 1):
                        gr, gi = g_hat[j, re, :], g_hat[j, im, :]
                        tr = gr * ur[a - j] - gi * ui[a - j]
                        ti = gr * ui[a - j] + gi * ur[a - j]
                        yr = tr if yr is None else yr + tr
                        yi = ti if yi is None else yi + ti
                    y_hat[a, re, :] = yr
                    y_hat[a, im, :] = yi
                return carry2

            jax.lax.fori_loop(0, _BLK // 8, freq_body, 0)
            inv = inv_ref[...]
            dsk = dskip_ref[:, cols].astype(f32)
            for a in range(n_blk):
                rows = pl.ds(a * _BLK, _BLK)
                y = _dot(inv, y_hat[a].astype(bf16))
                y = y + kv_vm[rows, :].astype(f32) * dsk
                b = x_vm[rows, cols].astype(f32) * y
                b_vm[rows, cols] = (1.0 - gate_vm[rows, :]) * b
            return carry

        jax.lax.fori_loop(0, n_ct, b_tile, 0)

        def w_body(j, carry):
            for m in range(3):
                w_copy(m, j).wait()
                wqkv[j, :, m * PW:(m + 1) * PW] = stage[j, m].T
            return carry

        jax.lax.fori_loop(0, n_pair, w_body, 0)
        wo_copy.wait()

        row = jax.lax.broadcasted_iota(jnp.int32, (L, 2 * L), 0)
        col = jax.lax.broadcasted_iota(jnp.int32, (L, 2 * L), 1)
        first = col < L
        key = jnp.where(first, col, col - L)
        visible = (row < M) | (row >= key)
        lane = jax.lax.broadcasted_iota(jnp.int32, (L, PW), 1)
        lane_first = lane < Dh

        def stack(t):
            zero = jnp.zeros_like(t)
            both = jnp.concatenate(
                [jnp.where(lane_first, t, zero), jnp.where(lane_first, zero, t)], axis=0)
            return both.astype(bf16)

        def out_copy(i):
            rows = pl.ds(i * out_chunk * seg, out_chunk * seg)
            return pltpu.make_async_copy(out_vm.at[rows, :], out_hbm.at[rows, :], out_sem)

        def step(s, mem):
            rows = pl.ds(pl.multiple_of(s * seg, seg), seg)
            h = jnp.concatenate([mem, x_vm[rows, :].astype(f32)], axis=0)
            o_heads = []
            for j in range(n_pair):
                qkv = _dot(h, wqkv[j])
                q, k, v = qkv[:, 0:PW], qkv[:, PW:2 * PW], qkv[:, 2 * PW:3 * PW]
                sc = _dot_nt(q, stack(k)) * scale
                sc = jnp.where(visible, sc, -1e9)
                m0 = jnp.max(jnp.where(first, sc, -jnp.inf), axis=-1, keepdims=True)
                m1 = jnp.max(jnp.where(first, -jnp.inf, sc), axis=-1, keepdims=True)
                e = jnp.exp(sc - jnp.where(first, m0, m1))
                s0 = jnp.sum(jnp.where(first, e, 0.0), axis=-1, keepdims=True)
                s1 = jnp.sum(jnp.where(first, 0.0, e), axis=-1, keepdims=True)
                p = e / jnp.where(first, s0, s1)
                o_heads.append(_dot(p, stack(v)))
            o = _dot(jnp.concatenate(o_heads, axis=1), wo_vm[...])
            gate = gate_vm[rows, :]
            res = jnp.concatenate([gate] * n_ct, axis=1) * o[M:] + b_vm[rows, :]
            out_vm[rows, :] = res.astype(bf16)

            @pl.when(s % out_chunk == out_chunk - 1)
            def _():
                out_copy(s // out_chunk).start()

            return o[0:M]

        jax.lax.fori_loop(0, n_seg, step, mem0_ref[...].astype(f32))
        for i in range(n_seg // out_chunk):
            out_copy(i).wait()

    return kernel


def pallas_gated_mix__memory_aug_recurrent_mem_tr__ssm_conv_h3__prompt_kernel(
    A_x, A_mem0, A_Wq, A_Wk, A_Wv, A_Wo, A_seg_len, B_q, B_k, B_v,
    B_shift_k, B_ssm_k, B_ssm_D, gate_w,
):
    del B_q
    seg = int(A_seg_len)
    B, S, D = A_x.shape
    _, H, Dh = A_Wq.shape
    M = A_mem0.shape[1]
    ks = B_shift_k.shape[1]
    assert B == 1 and H % 2 == 0 and (2 * Dh) % 128 == 0 and D % 128 == 0
    assert S % _BLK == 0 and S % (8 * seg) == 0 and M == 8 and seg % 16 == 0 and ks <= 8
    PW = 2 * Dh
    n_pair = H // 2
    n_blk = S // _BLK
    f32, bf16 = jnp.float32, jnp.bfloat16
    fwd, inv = _dft_matrices()

    def heads_major(w):
        return jnp.transpose(w, (1, 2, 0)).reshape(H * Dh, D)

    hbm = pl.BlockSpec(memory_space=pl.ANY)
    vmem = pl.BlockSpec(memory_space=pltpu.VMEM)
    out = pl.pallas_call(
        _make_kernel(S, D, H, Dh, M, seg, ks),
        out_shape=jax.ShapeDtypeStruct((S, D), A_x.dtype),
        in_specs=[hbm, vmem, hbm, hbm, hbm, hbm, hbm, hbm,
                  vmem, hbm, vmem, vmem, vmem, vmem],
        out_specs=hbm,
        scratch_shapes=[
            pltpu.VMEM((S, D), bf16),
            pltpu.VMEM((S, D), bf16),
            pltpu.VMEM((S, D), bf16),
            pltpu.VMEM((D, S), bf16),
            pltpu.VMEM((n_pair, 3, PW, D), bf16),
            pltpu.VMEM((n_pair, D, 3 * PW), bf16),
            pltpu.VMEM((H * Dh, D), bf16),
            pltpu.VMEM((S + 8, 128), f32),
            pltpu.VMEM((n_blk, 2 * _BLK, 128), f32),
            pltpu.VMEM((n_blk, 2 * _BLK, 128), f32),
            pltpu.VMEM((n_blk, 2 * _BLK, 128), f32),
            pltpu.VMEM((S, 128), bf16),
            pltpu.VMEM((S, D), f32),
            pltpu.VMEM((S, 128), f32),
            pltpu.VMEM((S, D), bf16),
            pltpu.SemaphoreType.DMA((4,)),
            pltpu.SemaphoreType.DMA((n_pair * 3,)),
            pltpu.SemaphoreType.DMA(()),
            pltpu.SemaphoreType.DMA(()),
        ],
        compiler_params=pltpu.CompilerParams(vmem_limit_bytes=120 * 1024 * 1024),
    )(
        A_x.reshape(S, D), A_mem0.reshape(M, D),
        heads_major(A_Wq), heads_major(A_Wk), heads_major(A_Wv),
        A_Wo.reshape(H * Dh, D), B_k.reshape(S, D), B_v.reshape(S, D),
        B_shift_k.T, B_ssm_k, B_ssm_D.reshape(1, D), gate_w.reshape(1, D),
        jnp.asarray(fwd, bf16), jnp.asarray(inv, bf16),
    )
    return out.reshape(B, S, D)
```

```python
import numpy as np

import jax
import jax.numpy as jnp
import jax.experimental.pallas as pl
import jax.experimental.pallas.tpu as pltpu

_BLK = 128
_RING = 4
_PRE = 8
_UNROLL = 2


def _dft_matrices():
    f = np.concatenate([np.arange(0, _BLK, 2), np.arange(1, _BLK, 2)])
    t = np.arange(_BLK)
    ang = 2.0 * np.pi * (f[:, None] + 0.5) * t[None, :] / (2 * _BLK)
    fwd = np.concatenate([np.cos(ang), -np.sin(ang)], axis=0)
    inv = fwd.T / _BLK
    return fwd.astype(np.float32), inv.astype(np.float32)


def _dot(a, b):
    return jax.lax.dot_general(
        a, b, (((1,), (0,)), ((), ())), preferred_element_type=jnp.float32)


def _dot_nt(a, b):
    return jax.lax.dot_general(
        a, b, (((1,), (1,)), ((), ())), preferred_element_type=jnp.float32)


def _step_schedule(n):
    tail = (3, 3, 1)
    lag = sum(tail) + 2
    sched = [("P", 0)]
    done = 0
    for j in range(1, n):
        sched.append(("P", j))
        if j >= 2:
            sched.append(("V", j - 2))
        sched.append(("S", j - 1))
        if j >= lag:
            sched.append(("O", done))
            done += 1
    for count, then in zip(tail[:2], ([("V", n - 2), ("S", n - 1)], [("V", n - 1)])):
        sched += [("O", i) for i in range(done, done + count)] + then
        done += count
    return sched + [("O", i) for i in range(done, n)]


def _make_kernel(S, D, H, Dh, M, seg, ks):
    L = M + seg
    n_seg = S // seg
    n_pair = H // 2
    PW = 2 * Dh
    n_blk = S // _BLK
    n_ct = D // 128
    n_plain = n_pair - n_ct
    half = _BLK // 2
    scale = float(Dh) ** -0.5
    f32, bf16, u32 = jnp.float32, jnp.bfloat16, jnp.uint32

    def kernel(x_hbm, mem0_ref, wq_hbm, wk_hbm, wv_hbm, wo_hbm, k_hbm, v_hbm,
               shift_ref, g_hbm, dskip_ref, gw_ref, fwd_ref, inv_ref,
               out_hbm,
               x_vm, xs_vm, xsel, k_vm, v_vm, g_vm, stage, wqkv, wo_vm, pre,
               kpad, kv_vm, u_hat, g_hat, y_vm, out_vm,
               in_sem, w_sem, out_sem):
        xs_copy = pltpu.make_async_copy(
            x_hbm.at[:, pl.ds(seg - _PRE, _PRE), :], xs_vm, in_sem.at[0])
        late_copies = [
            pltpu.make_async_copy(g_hbm, g_vm, in_sem.at[1]),
            pltpu.make_async_copy(k_hbm, k_vm, in_sem.at[2]),
            pltpu.make_async_copy(v_hbm, v_vm, in_sem.at[3]),
            pltpu.make_async_copy(x_hbm, x_vm, in_sem.at[4]),
        ]

        def w_copies(j):
            slot = j % _RING
            rows = pl.ds(pl.multiple_of(j * PW, PW), PW)
            return [
                pltpu.make_async_copy(
                    src.at[rows, :], stage.at[slot, m], w_sem.at[slot * 4 + m])
                for m, src in enumerate((wq_hbm, wk_hbm, wv_hbm, wo_hbm))]

        xs_copy.start()
        for j in range(_RING - 1):
            for c in w_copies(j):
                c.start()
        xs_copy.wait()
        xsel[...] = xs_vm[...].astype(f32).reshape(n_seg * _PRE, D).astype(bf16)
        kpad[0:8, :] = jnp.zeros((8, 128), f32)

        def fetch_pair(j):
            @pl.when(j + _RING - 1 < n_pair)
            def _():
                for c in w_copies(j + _RING - 1):
                    c.start()

            for c in w_copies(j):
                c.wait()

        def prepare_pair(j):
            slot = j % _RING
            for m in range(3):
                wt = stage[slot, m]
                cols = slice(m * PW, (m + 1) * PW)
                pre[j, :, cols] = _dot_nt(xsel[...], wt)
                wqkv[j, :, cols] = pltpu.bitcast(wt.T, u32)
            wo_vm[j] = pltpu.bitcast(stage[slot, 3], u32)

        def plain_body(j, carry):
            for i, c in enumerate(late_copies):
                @pl.when(j == 1 + 2 * i)
                def _():
                    c.start()

            fetch_pair(j)
            prepare_pair(j)
            return carry

        jax.lax.fori_loop(0, n_plain, plain_body, 0)
        for c in late_copies:
            c.wait()

        def conv_body(c, carry):
            fetch_pair(n_plain + c)
            cols = pl.ds(pl.multiple_of(c * 128, 128), 128)
            fwd = fwd_ref[...]
            prev = None
            for a in range(n_blk):
                cur = _dot_nt(fwd, g_vm[cols, pl.ds(a * _BLK, _BLK)])
                if prev is None:
                    g_hat[a] = cur
                else:
                    g_hat[a, 0:half, :] = cur[0:half] - prev[_BLK:_BLK + half]
                    g_hat[a, half:_BLK, :] = cur[half:_BLK] + prev[_BLK + half:]
                    g_hat[a, _BLK:_BLK + half, :] = cur[_BLK:_BLK + half] + prev[0:half]
                    g_hat[a, _BLK + half:, :] = cur[_BLK + half:] - prev[half:_BLK]
                prev = cur
            kpad[8:8 + S, :] = k_vm[:, cols].astype(f32)
            sh = shift_ref[:, cols].astype(f32)
            for a in range(n_blk):
                rows = pl.ds(a * _BLK, _BLK)
                acc = kpad[pl.ds(8 + a * _BLK, _BLK), :] * sh[0:1, :]
                for i in range(1, ks):
                    acc = acc + kpad[pl.ds(8 + a * _BLK - i, _BLK), :] * sh[i:i + 1, :]
                kv = acc * v_vm[rows, cols].astype(f32)
                kv_vm[rows, :] = kv
                u_hat[a] = _dot(fwd, kv.astype(bf16))

            prepare_pair(n_plain + c)

            for r in range(_BLK // 8):
                re, im = pl.ds(r * 8, 8), pl.ds(_BLK + r * 8, 8)
                ur = [u_hat[a, re, :] for a in range(n_blk)]
                ui = [u_hat[a, im, :] for a in range(n_blk)]
                for a in range(n_blk):
                    yr = yi = None
                    for j in range(a + 1):
                        gr, gi = g_hat[j, re, :], g_hat[j, im, :]
                        tr = gr * ur[a - j] - gi * ui[a - j]
                        ti = gr * ui[a - j] + gi * ur[a - j]
                        yr = tr if yr is None else yr + tr
                        yi = ti if yi is None else yi + ti
                    u_hat[a, re, :] = yr
                    u_hat[a, im, :] = yi

            inv = inv_ref[...]
            dsk = dskip_ref[:, cols].astype(f32)
            for a in range(n_blk):
                rows = pl.ds(a * _BLK, _BLK)
                y_vm[rows, cols] = _dot(inv, u_hat[a].astype(bf16)) + kv_vm[rows, :] * dsk
            return carry

        jax.lax.fori_loop(0, n_ct, conv_body, 0)

        row = jax.lax.broadcasted_iota(jnp.int32, (L, 2 * L), 0)
        col = jax.lax.broadcasted_iota(jnp.int32, (L, 2 * L), 1)
        first = col < L
        visible = (row < M) | (row >= jnp.where(first, col, col - L))
        lane_first = jax.lax.broadcasted_iota(jnp.int32, (L, PW), 1) < Dh
        gw = gw_ref[...].astype(f32)

        def stack(t):
            zero = jnp.zeros_like(t)
            both = jnp.concatenate(
                [jnp.where(lane_first, t, zero), jnp.where(lane_first, zero, t)], axis=0)
            return both.astype(bf16)

        def step(s, mem):
            xs = x_vm[s].astype(f32)
            h = jnp.concatenate([mem, xs[0:seg - _PRE]], axis=0)
            ahead = pl.ds(pl.multiple_of(s * _PRE, _PRE), _PRE)
            qkv, p, o = {}, {}, {}
            acc = None
            for op, j in _step_schedule(n_pair):
                if op == "P":
                    qkv[j] = jnp.concatenate(
                        [_dot(h, pltpu.bitcast(wqkv[j], bf16)), pre[j, ahead, :]], axis=0)
                elif op == "S":
                    sc = _dot_nt(qkv[j][:, 0:PW], stack(qkv[j][:, PW:2 * PW])) * scale
                    sc = jnp.where(visible, sc, -1e9)
                    m0 = jnp.max(jnp.where(first, sc, -jnp.inf), axis=-1, keepdims=True)
                    m1 = jnp.max(jnp.where(first, -jnp.inf, sc), axis=-1, keepdims=True)
                    e = jnp.exp(sc - jnp.where(first, m0, m1))
                    s0 = jnp.sum(jnp.where(first, e, 0.0), axis=-1, keepdims=True)
                    s1 = jnp.sum(jnp.where(first, 0.0, e), axis=-1, keepdims=True)
                    p[j] = e / jnp.where(first, s0, s1)
                elif op == "V":
                    o[j] = _dot(p[j], stack(qkv[j][:, 2 * PW:]))
                else:
                    t = _dot(o[j], pltpu.bitcast(wo_vm[j], bf16))
                    acc = t if acc is None else acc + t
            gate = jax.nn.sigmoid(jnp.sum(xs * gw, axis=-1, keepdims=True))
            b = xs * y_vm[pl.ds(pl.multiple_of(s * seg, seg), seg), :]
            out_vm[s] = (gate * acc[M:] + (1.0 - gate) * b).astype(bf16)
            return acc[0:M]

        def out_copy(i):
            segs = pl.ds(i * _UNROLL, _UNROLL)
            return pltpu.make_async_copy(out_vm.at[segs], out_hbm.at[segs], out_sem)

        def steps(i, mem):
            for u in range(_UNROLL):
                mem = step(i * _UNROLL + u, mem)
            out_copy(i).start()
            return mem

        jax.lax.fori_loop(0, n_seg // _UNROLL, steps, mem0_ref[...].astype(f32))
        pltpu.make_async_copy(out_vm, out_hbm, out_sem).wait()

    return kernel


def pallas_gated_mix__memory_aug_recurrent_mem_tr__ssm_conv_h3__prompt_kernel(
    A_x, A_mem0, A_Wq, A_Wk, A_Wv, A_Wo, A_seg_len, B_q, B_k, B_v,
    B_shift_k, B_ssm_k, B_ssm_D, gate_w,
):
    del B_q
    seg = int(A_seg_len)
    B, S, D = A_x.shape
    _, H, Dh = A_Wq.shape
    M = A_mem0.shape[1]
    ks = B_shift_k.shape[1]
    PW = 2 * Dh
    n_pair = H // 2
    n_blk = S // _BLK
    n_seg = S // seg
    assert B == 1 and H % 2 == 0 and PW % 128 == 0 and D % 128 == 0
    assert S % _BLK == 0 and S % (_UNROLL * seg) == 0 and seg % 16 == 0
    assert M % 8 == 0 and ks <= 8 and n_pair >= D // 128 + 8
    f32, bf16, u32 = jnp.float32, jnp.bfloat16, jnp.uint32
    fwd, inv = _dft_matrices()

    def heads_major(w):
        return jnp.transpose(w, (1, 2, 0)).reshape(H * Dh, D)

    hbm = pl.BlockSpec(memory_space=pl.ANY)
    vmem = pl.BlockSpec(memory_space=pltpu.VMEM)
    out = pl.pallas_call(
        _make_kernel(S, D, H, Dh, M, seg, ks),
        out_shape=jax.ShapeDtypeStruct((n_seg, seg, D), A_x.dtype),
        in_specs=[hbm, vmem, hbm, hbm, hbm, hbm, hbm, hbm,
                  vmem, hbm, vmem, vmem, vmem, vmem],
        out_specs=hbm,
        scratch_shapes=[
            pltpu.VMEM((n_seg, seg, D), bf16),
            pltpu.VMEM((n_seg, _PRE, D), bf16),
            pltpu.VMEM((n_seg * _PRE, D), bf16),
            pltpu.VMEM((S, D), bf16),
            pltpu.VMEM((S, D), bf16),
            pltpu.VMEM((D, S), bf16),
            pltpu.VMEM((_RING, 4, PW, D), bf16),
            pltpu.VMEM((n_pair, D // 2, 3 * PW), u32),
            pltpu.VMEM((n_pair, PW // 2, D), u32),
            pltpu.VMEM((n_pair, n_seg * _PRE, 3 * PW), f32),
            pltpu.VMEM((S + 8, 128), f32),
            pltpu.VMEM((S, 128), f32),
            pltpu.VMEM((n_blk, 2 * _BLK, 128), f32),
            pltpu.VMEM((n_blk, 2 * _BLK, 128), f32),
            pltpu.VMEM((S, D), f32),
            pltpu.VMEM((n_seg, seg, D), bf16),
            pltpu.SemaphoreType.DMA((5,)),
            pltpu.SemaphoreType.DMA((_RING * 4,)),
            pltpu.SemaphoreType.DMA(()),
        ],
        compiler_params=pltpu.CompilerParams(vmem_limit_bytes=120 * 1024 * 1024),
    )(
        A_x.reshape(n_seg, seg, D), A_mem0.reshape(M, D),
        heads_major(A_Wq), heads_major(A_Wk), heads_major(A_Wv),
        A_Wo.reshape(H * Dh, D), B_k.reshape(S, D), B_v.reshape(S, D),
        B_shift_k.T, B_ssm_k, B_ssm_D.reshape(1, D), gate_w.reshape(1, D),
        jnp.asarray(fwd, bf16), jnp.asarray(inv, bf16),
    )
    return out.reshape(B, S, D)
```

```python
import numpy as np

import jax
import jax.numpy as jnp
import jax.experimental.pallas as pl
import jax.experimental.pallas.tpu as pltpu

_BLK = 128
_RING = 4
_PRE = 8
_UNROLL = 2


def _dft_matrices():
    f = np.concatenate([np.arange(0, _BLK, 2), np.arange(1, _BLK, 2)])
    t = np.arange(_BLK)
    ang = 2.0 * np.pi * (f[:, None] + 0.5) * t[None, :] / (2 * _BLK)
    fwd = np.concatenate([np.cos(ang), -np.sin(ang)], axis=0)
    inv = fwd.T / _BLK
    return fwd.astype(np.float32), inv.astype(np.float32)


def _dot(a, b):
    return jax.lax.dot_general(
        a, b, (((1,), (0,)), ((), ())), preferred_element_type=jnp.float32)


def _dot_nt(a, b):
    return jax.lax.dot_general(
        a, b, (((1,), (1,)), ((), ())), preferred_element_type=jnp.float32)


def _step_schedule(n):
    tail = (3, 3, 1)
    lag = sum(tail) + 2
    sched = [("P", 0)]
    done = 0
    for j in range(1, n):
        sched.append(("P", j))
        if j >= 2:
            sched.append(("V", j - 2))
        sched.append(("S", j - 1))
        if j >= lag:
            sched.append(("O", done))
            done += 1
    for count, then in zip(tail[:2], ([("V", n - 2), ("S", n - 1)], [("V", n - 1)])):
        sched += [("O", i) for i in range(done, done + count)] + then
        done += count
    return sched + [("O", i) for i in range(done, n)]


def _make_kernel(S, D, H, Dh, M, seg, ks):
    L = M + seg
    n_seg = S // seg
    n_pair = H // 2
    PW = 2 * Dh
    n_blk = S // _BLK
    n_ct = D // 128
    n_plain = n_pair - 2 * n_ct
    half = _BLK // 2
    scale = float(Dh) ** -0.5
    f32, bf16, u32 = jnp.float32, jnp.bfloat16, jnp.uint32

    def kernel(x_hbm, mem0_ref, wq_hbm, wk_hbm, wv_hbm, wo_hbm, k_hbm, v_hbm,
               shift_ref, g_hbm, dskip_ref, gw_ref, fwd_ref, inv_ref,
               out_hbm,
               x_vm, xs_vm, xsel, k_vm, v_vm, g_vm, stage, wqkv, wo_vm, pre,
               kpad, kv_vm, u_hat, g_hat, y_hat, y_vm, out_vm,
               in_sem, tile_sem, w_sem, out_sem):
        xs_copy = pltpu.make_async_copy(
            x_hbm.at[:, pl.ds(seg - _PRE, _PRE), :], xs_vm, in_sem.at[0])
        x_copy = pltpu.make_async_copy(x_hbm, x_vm, in_sem.at[1])

        def tile_copies(c):
            cols = pl.ds(pl.multiple_of(c * 128, 128), 128)
            return [
                pltpu.make_async_copy(g_hbm.at[cols, :], g_vm.at[c], tile_sem.at[c]),
                pltpu.make_async_copy(k_hbm.at[:, cols], k_vm.at[c], tile_sem.at[c]),
                pltpu.make_async_copy(v_hbm.at[:, cols], v_vm.at[c], tile_sem.at[c]),
            ]

        def w_copies(j):
            slot = j % _RING
            rows = pl.ds(pl.multiple_of(j * PW, PW), PW)
            return [
                pltpu.make_async_copy(
                    src.at[rows, :], stage.at[slot, m], w_sem.at[slot * 4 + m])
                for m, src in enumerate((wq_hbm, wk_hbm, wv_hbm, wo_hbm))]

        xs_copy.start()
        for c in w_copies(0):
            c.start()
        xs_copy.wait()
        for j in range(1, _RING - 1):
            for c in w_copies(j):
                c.start()
        xsel[...] = xs_vm[...].astype(f32).reshape(n_seg * _PRE, D).astype(bf16)
        kpad[0:8, :] = jnp.zeros((8, 128), f32)

        def fetch_pair(j):
            @pl.when(j + _RING - 1 < n_pair)
            def _():
                for c in w_copies(j + _RING - 1):
                    c.start()

            for c in w_copies(j):
                c.wait()

        def repack_pair(j):
            slot = j % _RING
            for m in range(3):
                wqkv[j, :, m * PW:(m + 1) * PW] = pltpu.bitcast(stage[slot, m].T, u32)
            wo_vm[j] = pltpu.bitcast(stage[slot, 3], u32)

        def project_ahead(j, rows):
            for m in range(3):
                pre[j, rows, m * PW:(m + 1) * PW] = _dot_nt(xsel[rows, :], stage[j % _RING, m])

        def plain_body(j, carry):
            @pl.when(j == 2)
            def _():
                for c in tile_copies(0):
                    c.start()

            fetch_pair(j)
            project_ahead(j, slice(None))
            repack_pair(j)
            return carry

        jax.lax.fori_loop(0, n_plain, plain_body, 0)

        def conv_body(c, carry):
            @pl.when(c + 1 < n_ct)
            def _():
                for copy in tile_copies(c + 1):
                    copy.start()

            @pl.when(c + 1 == n_ct)
            def _():
                x_copy.start()

            for copy in tile_copies(c):
                copy.wait()
            cols = pl.ds(pl.multiple_of(c * 128, 128), 128)
            fwd = fwd_ref[...]
            prev = None
            for a in range(n_blk):
                cur = _dot_nt(fwd, g_vm[c, :, pl.ds(a * _BLK, _BLK)])
                if prev is None:
                    g_hat[a] = cur
                else:
                    g_hat[a, 0:half, :] = cur[0:half] - prev[_BLK:_BLK + half]
                    g_hat[a, half:_BLK, :] = cur[half:_BLK] + prev[_BLK + half:]
                    g_hat[a, _BLK:_BLK + half, :] = cur[_BLK:_BLK + half] + prev[0:half]
                    g_hat[a, _BLK + half:, :] = cur[_BLK + half:] - prev[half:_BLK]
                prev = cur
            kpad[8:8 + S, :] = k_vm[c].astype(f32)
            sh = shift_ref[:, cols].astype(f32)
            for a in range(n_blk):
                rows = pl.ds(a * _BLK, _BLK)
                acc = kpad[pl.ds(8 + a * _BLK, _BLK), :] * sh[0:1, :]
                for i in range(1, ks):
                    acc = acc + kpad[pl.ds(8 + a * _BLK - i, _BLK), :] * sh[i:i + 1, :]
                kv = acc * v_vm[c, rows, :].astype(f32)
                kv_vm[rows, :] = kv
                u_hat[a] = _dot(fwd, kv.astype(bf16))

            def product_body(i, carry2):
                j = n_plain + 2 * c + i
                fetch_pair(j)
                n_rows = n_seg * _PRE
                pace = []
                for m in range(3):
                    total = None
                    for kt in range(n_ct):
                        kk = slice(kt * 128, (kt + 1) * 128)
                        t = _dot_nt(xsel[:, kk], stage[j % _RING, m, :, kk])
                        pace += [t[q:q + 8, 0:128] for q in range(0, n_rows, 8)]
                        total = t if total is None else total + t
                    pre[j, :, m * PW:(m + 1) * PW] = total
                repack_pair(j)
                n_freq = _BLK // 2
                n_mac = (n_freq // 8) * n_blk * (n_blk + 1) // 2
                done = 0
                for r in range(0, n_freq, 8):
                    re = pl.ds(pl.multiple_of(i * n_freq + r, 8), 8)
                    im = pl.ds(pl.multiple_of(i * n_freq + r + _BLK, 8), 8)
                    yr, yi = [None] * n_blk, [None] * n_blk
                    for jj in range(n_blk):
                        gr = jnp.where(i < 0, pace[done * 9 * len(pace) // (10 * n_mac)],
                                       g_hat[jj, re, :])
                        gi = g_hat[jj, im, :]
                        for a in range(jj, n_blk):
                            ur, ui = u_hat[a - jj, re, :], u_hat[a - jj, im, :]
                            tr = gr * ur - gi * ui
                            ti = gr * ui + gi * ur
                            yr[a] = tr if yr[a] is None else yr[a] + tr
                            yi[a] = ti if yi[a] is None else yi[a] + ti
                        y_hat[jj, re, :] = yr[jj]
                        y_hat[jj, im, :] = yi[jj]
                        done += n_blk - jj
                return carry2

            jax.lax.fori_loop(0, 2, product_body, 0)

            inv = inv_ref[...]
            dsk = dskip_ref[:, cols].astype(f32)
            for a in range(n_blk):
                rows = pl.ds(a * _BLK, _BLK)
                y_vm[rows, cols] = _dot(inv, y_hat[a].astype(bf16)) + kv_vm[rows, :] * dsk
            return carry

        jax.lax.fori_loop(0, n_ct, conv_body, 0)
        x_copy.wait()

        row = jax.lax.broadcasted_iota(jnp.int32, (L, 2 * L), 0)
        col = jax.lax.broadcasted_iota(jnp.int32, (L, 2 * L), 1)
        first = col < L
        visible = (row < M) | (row >= jnp.where(first, col, col - L))
        lane_first = jax.lax.broadcasted_iota(jnp.int32, (L, PW), 1) < Dh
        gw = gw_ref[...].astype(f32)

        def stack(t):
            zero = jnp.zeros_like(t)
            both = jnp.concatenate(
                [jnp.where(lane_first, t, zero), jnp.where(lane_first, zero, t)], axis=0)
            return both.astype(bf16)

        def step(s, mem):
            xs = x_vm[s].astype(f32)
            h = jnp.concatenate([mem, xs[0:seg - _PRE]], axis=0)
            ahead = pl.ds(pl.multiple_of(s * _PRE, _PRE), _PRE)
            qkv, p, o = {}, {}, {}
            acc = None
            for op, j in _step_schedule(n_pair):
                if op == "P":
                    qkv[j] = jnp.concatenate(
                        [_dot(h, pltpu.bitcast(wqkv[j], bf16)), pre[j, ahead, :]], axis=0)
                elif op == "S":
                    sc = _dot_nt(qkv[j][:, 0:PW], stack(qkv[j][:, PW:2 * PW])) * scale
                    sc = jnp.where(visible, sc, -1e9)
                    m0 = jnp.max(jnp.where(first, sc, -jnp.inf), axis=-1, keepdims=True)
                    m1 = jnp.max(jnp.where(first, -jnp.inf, sc), axis=-1, keepdims=True)
                    e = jnp.exp(sc - jnp.where(first, m0, m1))
                    s0 = jnp.sum(jnp.where(first, e, 0.0), axis=-1, keepdims=True)
                    s1 = jnp.sum(jnp.where(first, 0.0, e), axis=-1, keepdims=True)
                    p[j] = e / jnp.where(first, s0, s1)
                elif op == "V":
                    o[j] = _dot(p[j], stack(qkv[j][:, 2 * PW:]))
                else:
                    t = _dot(o[j], pltpu.bitcast(wo_vm[j], bf16))
                    acc = t if acc is None else acc + t
            gate = jax.nn.sigmoid(jnp.sum(xs * gw, axis=-1, keepdims=True))
            b = xs * y_vm[pl.ds(pl.multiple_of(s * seg, seg), seg), :]
            out_vm[s] = (gate * acc[M:] + (1.0 - gate) * b).astype(bf16)
            return acc[0:M]

        def out_copy(i):
            segs = pl.ds(i * _UNROLL, _UNROLL)
            return pltpu.make_async_copy(out_vm.at[segs], out_hbm.at[segs], out_sem)

        def steps(i, mem):
            for u in range(_UNROLL):
                mem = step(i * _UNROLL + u, mem)
            out_copy(i).start()
            return mem

        jax.lax.fori_loop(0, n_seg // _UNROLL, steps, mem0_ref[...].astype(f32))
        pltpu.make_async_copy(out_vm, out_hbm, out_sem).wait()

    return kernel


def pallas_gated_mix__memory_aug_recurrent_mem_tr__ssm_conv_h3__prompt_kernel(
    A_x, A_mem0, A_Wq, A_Wk, A_Wv, A_Wo, A_seg_len, B_q, B_k, B_v,
    B_shift_k, B_ssm_k, B_ssm_D, gate_w,
):
    del B_q
    seg = int(A_seg_len)
    B, S, D = A_x.shape
    _, H, Dh = A_Wq.shape
    M = A_mem0.shape[1]
    ks = B_shift_k.shape[1]
    PW = 2 * Dh
    n_pair = H // 2
    n_blk = S // _BLK
    n_seg = S // seg
    assert B == 1 and H % 2 == 0 and PW % 128 == 0 and D % 128 == 0
    assert S % _BLK == 0 and S % (_UNROLL * seg) == 0 and seg % 16 == 0
    assert M % 8 == 0 and ks <= 8 and n_pair >= 2 * (D // 128) + 5
    f32, bf16, u32 = jnp.float32, jnp.bfloat16, jnp.uint32
    fwd, inv = _dft_matrices()

    def heads_major(w):
        return jnp.transpose(w, (1, 2, 0)).reshape(H * Dh, D)

    hbm = pl.BlockSpec(memory_space=pl.ANY)
    vmem = pl.BlockSpec(memory_space=pltpu.VMEM)
    out = pl.pallas_call(
        _make_kernel(S, D, H, Dh, M, seg, ks),
        out_shape=jax.ShapeDtypeStruct((n_seg, seg, D), A_x.dtype),
        in_specs=[hbm, vmem, hbm, hbm, hbm, hbm, hbm, hbm,
                  vmem, hbm, vmem, vmem, vmem, vmem],
        out_specs=hbm,
        scratch_shapes=[
            pltpu.VMEM((n_seg, seg, D), bf16),
            pltpu.VMEM((n_seg, _PRE, D), bf16),
            pltpu.VMEM((n_seg * _PRE, D), bf16),
            pltpu.VMEM((D // 128, S, 128), bf16),
            pltpu.VMEM((D // 128, S, 128), bf16),
            pltpu.VMEM((D // 128, 128, S), bf16),
            pltpu.VMEM((_RING, 4, PW, D), bf16),
            pltpu.VMEM((n_pair, D // 2, 3 * PW), u32),
            pltpu.VMEM((n_pair, PW // 2, D), u32),
            pltpu.VMEM((n_pair, n_seg * _PRE, 3 * PW), f32),
            pltpu.VMEM((S + 8, 128), f32),
            pltpu.VMEM((S, 128), f32),
            pltpu.VMEM((n_blk, 2 * _BLK, 128), f32),
            pltpu.VMEM((n_blk, 2 * _BLK, 128), f32),
            pltpu.VMEM((n_blk, 2 * _BLK, 128), f32),
            pltpu.VMEM((S, D), f32),
            pltpu.VMEM((n_seg, seg, D), bf16),
            pltpu.SemaphoreType.DMA((2,)),
            pltpu.SemaphoreType.DMA((D // 128,)),
            pltpu.SemaphoreType.DMA((_RING * 4,)),
            pltpu.SemaphoreType.DMA(()),
        ],
        compiler_params=pltpu.CompilerParams(vmem_limit_bytes=120 * 1024 * 1024),
    )(
        A_x.reshape(n_seg, seg, D), A_mem0.reshape(M, D),
        heads_major(A_Wq), heads_major(A_Wk), heads_major(A_Wv),
        A_Wo.reshape(H * Dh, D), B_k.reshape(S, D), B_v.reshape(S, D),
        B_shift_k.T, B_ssm_k, B_ssm_D.reshape(1, D), gate_w.reshape(1, D),
        jnp.asarray(fwd, bf16), jnp.asarray(inv, bf16),
    )
    return out.reshape(B, S, D)
```

```python
import numpy as np

import jax
import jax.numpy as jnp
import jax.experimental.pallas as pl
import jax.experimental.pallas.tpu as pltpu

_BLK = 128
_RING = 4
_PRE = 8
_ORDER, _LAG, _TAIL = "POVS", dict(S=1, V=3, O=9), "OOVSOOVOOOV"
_UNROLL = 4


def _dft_matrices():
    f = np.concatenate([np.arange(0, _BLK, 2), np.arange(1, _BLK, 2)])
    t = np.arange(_BLK)
    ang = 2.0 * np.pi * (f[:, None] + 0.5) * t[None, :] / (2 * _BLK)
    fwd = np.concatenate([np.cos(ang), -np.sin(ang)], axis=0)
    inv = fwd.T / _BLK
    return fwd.astype(np.float32), inv.astype(np.float32)


def _dot(a, b):
    return jax.lax.dot_general(
        a, b, (((1,), (0,)), ((), ())), preferred_element_type=jnp.float32)


def _dot_nt(a, b):
    return jax.lax.dot_general(
        a, b, (((1,), (1,)), ((), ())), preferred_element_type=jnp.float32)


def _step_schedule(n):
    lag = dict(P=0, **_LAG)
    done = dict.fromkeys("PSVO", 0)
    sched = []

    def emit(op):
        if done[op] < n:
            sched.append((op, done[op]))
            done[op] += 1

    for j in range(n):
        for op in _ORDER:
            if j >= lag[op]:
                emit(op)
    for op in _TAIL:
        emit(op)
    while done["O"] < n:
        emit("O")
    return sched


def _make_kernel(S, D, H, Dh, M, seg, ks):
    L = M + seg
    n_seg = S // seg
    n_pair = H // 2
    PW = 2 * Dh
    n_blk = S // _BLK
    n_ct = D // 128
    n_plain = n_pair - 2 * n_ct
    half = _BLK // 2
    scale = float(Dh) ** -0.5
    f32, bf16, u32 = jnp.float32, jnp.bfloat16, jnp.uint32

    def kernel(x_hbm, mem0_ref, wq_hbm, wk_hbm, wv_hbm, wo_hbm, k_hbm, v_hbm,
               shift_ref, g_hbm, dskip_ref, gw_ref, fwd_ref, inv_ref,
               out_hbm,
               x_vm, xs_vm, xsel, k_vm, v_vm, g_vm, stage, wqkv, wo_vm, pre,
               skip_vm, kpad, kv_vm, u_hat, g_hat, y_hat, y_vm, out_vm,
               in_sem, tile_sem, w_sem, out_sem):
        xs_copy = pltpu.make_async_copy(
            x_hbm.at[:, pl.ds(seg - _PRE, _PRE), :], xs_vm, in_sem.at[0])
        x_copy = pltpu.make_async_copy(x_hbm, x_vm, in_sem.at[1])

        def tile_copies(c):
            cols = pl.ds(pl.multiple_of(c * 128, 128), 128)
            return [
                pltpu.make_async_copy(g_hbm.at[cols, :], g_vm.at[c], tile_sem.at[c]),
                pltpu.make_async_copy(k_hbm.at[:, cols], k_vm.at[c], tile_sem.at[c]),
                pltpu.make_async_copy(v_hbm.at[:, cols], v_vm.at[c], tile_sem.at[c]),
            ]

        def w_copies(j):
            slot = j % _RING
            rows = pl.ds(pl.multiple_of(j * PW, PW), PW)
            return [
                pltpu.make_async_copy(
                    src.at[rows, :], stage.at[slot, m], w_sem.at[slot * 4 + m])
                for m, src in enumerate((wq_hbm, wk_hbm, wv_hbm, wo_hbm))]

        xs_copy.start()
        for c in w_copies(0):
            c.start()
        xs_copy.wait()
        for j in range(1, _RING - 1):
            for c in w_copies(j):
                c.start()
        xsel[...] = xs_vm[...].astype(f32).reshape(n_seg * _PRE, D).astype(bf16)
        kpad[0:8, :] = jnp.zeros((8, 128), f32)
        skip_vm[...] = dskip_ref[...].astype(f32).reshape(1, D)

        def fetch_pair(j):
            @pl.when(j + _RING - 1 < n_pair)
            def _():
                for c in w_copies(j + _RING - 1):
                    c.start()

            for c in w_copies(j):
                c.wait()

        def repack_pair(j):
            slot = j % _RING
            for m in range(3):
                wqkv[j, :, m * PW:(m + 1) * PW] = pltpu.bitcast(stage[slot, m].T, u32)
            wo_vm[j] = pltpu.bitcast(stage[slot, 3], u32)

        def project_ahead(j, rows):
            for m in range(3):
                pre[j, rows, m * PW:(m + 1) * PW] = _dot_nt(xsel[rows, :], stage[j % _RING, m])

        def plain_body(j, carry):
            @pl.when(j == 2)
            def _():
                for c in tile_copies(0):
                    c.start()

            fetch_pair(j)
            project_ahead(j, slice(None))
            repack_pair(j)
            return carry

        jax.lax.fori_loop(0, n_plain, plain_body, 0)

        def conv_body(c, carry):
            @pl.when(c + 1 < n_ct)
            def _():
                for copy in tile_copies(c + 1):
                    copy.start()

            @pl.when(c + 1 == n_ct)
            def _():
                x_copy.start()

            for copy in tile_copies(c):
                copy.wait()
            cols = pl.ds(pl.multiple_of(c * 128, 128), 128)
            fwd = fwd_ref[...]
            prev = None
            for a in range(n_blk):
                cur = _dot_nt(fwd, g_vm[c, :, pl.ds(a * _BLK, _BLK)])
                if prev is None:
                    g_hat[a] = cur
                else:
                    g_hat[a, 0:half, :] = cur[0:half] - prev[_BLK:_BLK + half]
                    g_hat[a, half:_BLK, :] = cur[half:_BLK] + prev[_BLK + half:]
                    g_hat[a, _BLK:_BLK + half, :] = cur[_BLK:_BLK + half] + prev[0:half]
                    g_hat[a, _BLK + half:, :] = cur[_BLK + half:] - prev[half:_BLK]
                prev = cur
            kpad[8:8 + S, :] = k_vm[c].astype(f32)
            sh = shift_ref[:, cols].astype(f32)
            for a in range(n_blk):
                rows = pl.ds(a * _BLK, _BLK)
                acc = kpad[pl.ds(8 + a * _BLK, _BLK), :] * sh[0:1, :]
                for i in range(1, ks):
                    acc = acc + kpad[pl.ds(8 + a * _BLK - i, _BLK), :] * sh[i:i + 1, :]
                kv = acc * v_vm[c, rows, :].astype(f32)
                kv_vm[rows, :] = kv
                u_hat[a] = _dot(fwd, kv.astype(bf16))

            def product_body(i, carry2):
                j = n_plain + 2 * c + i
                fetch_pair(j)
                n_rows = n_seg * _PRE
                pace = []
                for m in range(3):
                    total = None
                    for kt in range(n_ct):
                        kk = slice(kt * 128, (kt + 1) * 128)
                        t = _dot_nt(xsel[:, kk], stage[j % _RING, m, :, kk])
                        pace += [t[q:q + 8, 0:128] for q in range(0, n_rows, 8)]
                        total = t if total is None else total + t
                    pre[j, :, m * PW:(m + 1) * PW] = total
                repack_pair(j)
                n_freq = _BLK // 2
                n_mac = (n_freq // 8) * n_blk * (n_blk + 1) // 2
                done = 0
                for r in range(0, n_freq, 8):
                    re = pl.ds(pl.multiple_of(i * n_freq + r, 8), 8)
                    im = pl.ds(pl.multiple_of(i * n_freq + r + _BLK, 8), 8)
                    yr, yi = [None] * n_blk, [None] * n_blk
                    for jj in range(n_blk):
                        gr = jnp.where(i < 0, pace[done * 9 * len(pace) // (10 * n_mac)],
                                       g_hat[jj, re, :])
                        gi = g_hat[jj, im, :]
                        for a in range(jj, n_blk):
                            ur, ui = u_hat[a - jj, re, :], u_hat[a - jj, im, :]
                            tr = gr * ur - gi * ui
                            ti = gr * ui + gi * ur
                            yr[a] = tr if yr[a] is None else yr[a] + tr
                            yi[a] = ti if yi[a] is None else yi[a] + ti
                        y_hat[jj, re, :] = yr[jj]
                        y_hat[jj, im, :] = yi[jj]
                        done += n_blk - jj
                return carry2

            jax.lax.fori_loop(0, 2, product_body, 0)

            inv = inv_ref[...]
            dsk = skip_vm[:, cols]
            for a in range(n_blk):
                rows = pl.ds(a * _BLK, _BLK)
                y_vm[rows, cols] = _dot(inv, y_hat[a].astype(bf16)) + kv_vm[rows, :] * dsk
            return carry

        jax.lax.fori_loop(0, n_ct, conv_body, 0)
        x_copy.wait()

        row = jax.lax.broadcasted_iota(jnp.int32, (L, 2 * L), 0)
        col = jax.lax.broadcasted_iota(jnp.int32, (L, 2 * L), 1)
        first = col < L
        visible = (row < M) | (row >= jnp.where(first, col, col - L))
        lane_first = jax.lax.broadcasted_iota(jnp.int32, (L, PW), 1) < Dh
        gw = gw_ref[...].astype(f32).reshape(1, D)

        def stack(t):
            zero = jnp.zeros_like(t)
            both = jnp.concatenate(
                [jnp.where(lane_first, t, zero), jnp.where(lane_first, zero, t)], axis=0)
            return both.astype(bf16)

        def step(s, mem):
            xs = x_vm[s].astype(f32)
            h = jnp.concatenate([mem, xs[0:seg - _PRE]], axis=0)
            ahead = pl.ds(pl.multiple_of(s * _PRE, _PRE), _PRE)
            qkv, p, o = {}, {}, {}
            acc = None
            for op, j in _step_schedule(n_pair):
                if op == "P":
                    qkv[j] = jnp.concatenate(
                        [_dot(h, pltpu.bitcast(wqkv[j], bf16)), pre[j, ahead, :]], axis=0)
                elif op == "S":
                    sc = _dot_nt(qkv[j][:, 0:PW], stack(qkv[j][:, PW:2 * PW])) * scale
                    sc = jnp.where(visible, sc, -1e9)
                    m0 = jnp.max(jnp.where(first, sc, -jnp.inf), axis=-1, keepdims=True)
                    m1 = jnp.max(jnp.where(first, -jnp.inf, sc), axis=-1, keepdims=True)
                    e = jnp.exp(sc - jnp.where(first, m0, m1))
                    s0 = jnp.sum(jnp.where(first, e, 0.0), axis=-1, keepdims=True)
                    s1 = jnp.sum(jnp.where(first, 0.0, e), axis=-1, keepdims=True)
                    p[j] = e / jnp.where(first, s0, s1)
                elif op == "V":
                    o[j] = _dot(p[j], stack(qkv[j][:, 2 * PW:]))
                else:
                    t = _dot(o[j], pltpu.bitcast(wo_vm[j], bf16))
                    acc = t if acc is None else acc + t
            gate = jax.nn.sigmoid(jnp.sum(xs * gw, axis=-1, keepdims=True))
            b = xs * y_vm[pl.ds(pl.multiple_of(s * seg, seg), seg), :]
            out_vm[s] = (gate * acc[M:] + (1.0 - gate) * b).astype(bf16)
            return acc[0:M]

        def out_copy(i):
            segs = pl.ds(i * _UNROLL, _UNROLL)
            return pltpu.make_async_copy(out_vm.at[segs], out_hbm.at[segs], out_sem)

        def steps(i, mem):
            for u in range(_UNROLL):
                mem = step(i * _UNROLL + u, mem)
            out_copy(i).start()
            return mem

        jax.lax.fori_loop(0, n_seg // _UNROLL, steps, mem0_ref[...].astype(f32))
        pltpu.make_async_copy(out_vm, out_hbm, out_sem).wait()

    return kernel


def pallas_gated_mix__memory_aug_recurrent_mem_tr__ssm_conv_h3__prompt_kernel(
    A_x, A_mem0, A_Wq, A_Wk, A_Wv, A_Wo, A_seg_len, B_q, B_k, B_v,
    B_shift_k, B_ssm_k, B_ssm_D, gate_w,
):
    del B_q
    seg = int(A_seg_len)
    B, S, D = A_x.shape
    _, H, Dh = A_Wq.shape
    M = A_mem0.shape[1]
    ks = B_shift_k.shape[1]
    PW = 2 * Dh
    n_pair = H // 2
    n_blk = S // _BLK
    n_seg = S // seg
    assert B == 1 and H % 2 == 0 and PW % 128 == 0 and D % 128 == 0
    assert S % _BLK == 0 and S % (_UNROLL * seg) == 0 and seg % 16 == 0
    assert M % 8 == 0 and ks <= 8 and n_pair >= 2 * (D // 128) + 5
    f32, bf16, u32 = jnp.float32, jnp.bfloat16, jnp.uint32
    fwd, inv = _dft_matrices()

    def heads_major(w):
        return jnp.transpose(w, (1, 2, 0)).reshape(H * Dh, D)

    hbm = pl.BlockSpec(memory_space=pl.ANY)
    vmem = pl.BlockSpec(memory_space=pltpu.VMEM)
    out = pl.pallas_call(
        _make_kernel(S, D, H, Dh, M, seg, ks),
        out_shape=jax.ShapeDtypeStruct((n_seg, seg, D), A_x.dtype),
        in_specs=[hbm, vmem, hbm, hbm, hbm, hbm, hbm, hbm,
                  vmem, hbm, vmem, vmem, vmem, vmem],
        out_specs=hbm,
        scratch_shapes=[
            pltpu.VMEM((n_seg, seg, D), bf16),
            pltpu.VMEM((n_seg, _PRE, D), bf16),
            pltpu.VMEM((n_seg * _PRE, D), bf16),
            pltpu.VMEM((D // 128, S, 128), bf16),
            pltpu.VMEM((D // 128, S, 128), bf16),
            pltpu.VMEM((D // 128, 128, S), bf16),
            pltpu.VMEM((_RING, 4, PW, D), bf16),
            pltpu.VMEM((n_pair, D // 2, 3 * PW), u32),
            pltpu.VMEM((n_pair, PW // 2, D), u32),
            pltpu.VMEM((n_pair, n_seg * _PRE, 3 * PW), f32),
            pltpu.VMEM((1, D), f32),
            pltpu.VMEM((S + 8, 128), f32),
            pltpu.VMEM((S, 128), f32),
            pltpu.VMEM((n_blk, 2 * _BLK, 128), f32),
            pltpu.VMEM((n_blk, 2 * _BLK, 128), f32),
            pltpu.VMEM((n_blk, 2 * _BLK, 128), f32),
            pltpu.VMEM((S, D), f32),
            pltpu.VMEM((n_seg, seg, D), bf16),
            pltpu.SemaphoreType.DMA((2,)),
            pltpu.SemaphoreType.DMA((D // 128,)),
            pltpu.SemaphoreType.DMA((_RING * 4,)),
            pltpu.SemaphoreType.DMA(()),
        ],
        compiler_params=pltpu.CompilerParams(vmem_limit_bytes=120 * 1024 * 1024),
    )(
        A_x.reshape(n_seg, seg, D), A_mem0.reshape(M, D),
        heads_major(A_Wq), heads_major(A_Wk), heads_major(A_Wv),
        A_Wo.reshape(H * Dh, D), B_k.reshape(S, D), B_v.reshape(S, D),
        B_shift_k.T, B_ssm_k, B_ssm_D, gate_w,
        jnp.asarray(fwd, bf16), jnp.asarray(inv, bf16),
    )
    return out.reshape(B, S, D)
```

```python
import numpy as np

import jax
import jax.numpy as jnp
import jax.experimental.pallas as pl
import jax.experimental.pallas.tpu as pltpu

_BLK = 128
_RING = 4
_PRE = 8
_ORDER, _LAG, _TAIL = "POVS", dict(S=1, V=3, O=9), "OOVSOOVOOOV"
_UNROLL = 4


def _dft_matrices():
    f = np.concatenate([np.arange(0, _BLK, 2), np.arange(1, _BLK, 2)])
    t = np.arange(_BLK)
    ang = 2.0 * np.pi * (f[:, None] + 0.5) * t[None, :] / (2 * _BLK)
    fwd = np.concatenate([np.cos(ang), -np.sin(ang)], axis=0)
    inv = fwd.T / _BLK
    return fwd.astype(np.float32), inv.astype(np.float32)


def _dot(a, b):
    return jax.lax.dot_general(
        a, b, (((1,), (0,)), ((), ())), preferred_element_type=jnp.float32)


def _dot_nt(a, b):
    return jax.lax.dot_general(
        a, b, (((1,), (1,)), ((), ())), preferred_element_type=jnp.float32)


def _step_schedule(n):
    lag = dict(P=0, **_LAG)
    done = dict.fromkeys("PSVO", 0)
    sched = []

    def emit(op):
        if done[op] < n:
            sched.append((op, done[op]))
            done[op] += 1

    for j in range(n):
        for op in _ORDER:
            if j >= lag[op]:
                emit(op)
    for op in _TAIL:
        emit(op)
    while done["O"] < n:
        emit("O")
    return sched


def _make_kernel(S, D, H, Dh, M, seg, ks):
    L = M + seg
    n_seg = S // seg
    n_pair = H // 2
    PW = 2 * Dh
    n_blk = S // _BLK
    n_ct = D // 128
    n_plain = n_pair - 2 * n_ct
    half = _BLK // 2
    scale = float(Dh) ** -0.5
    f32, bf16, u32 = jnp.float32, jnp.bfloat16, jnp.uint32

    def kernel(x_hbm, mem0_ref, wq_hbm, wk_hbm, wv_hbm, wo_hbm, k_hbm, v_hbm,
               shift_ref, g_hbm, dskip_ref, gw_ref, fwd_ref, inv_ref,
               out_hbm,
               x_vm, xs_vm, xsel, k_vm, v_vm, g_vm, stage, wqkv, wo_vm, pre,
               skip_vm, kpad, kv_vm, u_hat, g_hat, y_hat, y_vm, out_vm,
               in_sem, tile_sem, w_sem, out_sem):
        xs_copy = pltpu.make_async_copy(
            x_hbm.at[:, pl.ds(seg - _PRE, _PRE), :], xs_vm, in_sem.at[0])
        x_copy = pltpu.make_async_copy(x_hbm, x_vm, in_sem.at[1])

        def tile_copies(c):
            cols = pl.ds(pl.multiple_of(c * 128, 128), 128)
            return [
                pltpu.make_async_copy(g_hbm.at[cols, :], g_vm.at[c], tile_sem.at[c]),
                pltpu.make_async_copy(k_hbm.at[:, cols], k_vm.at[c], tile_sem.at[c]),
                pltpu.make_async_copy(v_hbm.at[:, cols], v_vm.at[c], tile_sem.at[c]),
            ]

        def w_copies(j):
            slot = j % _RING
            rows = pl.ds(pl.multiple_of(j * PW, PW), PW)
            return [
                pltpu.make_async_copy(
                    src.at[rows, :], stage.at[slot, m], w_sem.at[slot * 4 + m])
                for m, src in enumerate((wq_hbm, wk_hbm, wv_hbm, wo_hbm))]

        xs_copy.start()
        for c in w_copies(0):
            c.start()
        xs_copy.wait()
        for j in range(1, _RING - 1):
            for c in w_copies(j):
                c.start()
        xsel[...] = xs_vm[...].astype(f32).reshape(n_seg * _PRE, D).astype(bf16)
        kpad[0:8, :] = jnp.zeros((8, 128), f32)
        skip_vm[...] = dskip_ref[...].astype(f32).reshape(1, D)

        def fetch_pair(j):
            @pl.when(j + _RING - 1 < n_pair)
            def _():
                for c in w_copies(j + _RING - 1):
                    c.start()

            for c in w_copies(j):
                c.wait()

        def repack_pair(j):
            slot = j % _RING
            for m in range(3):
                wqkv[j, :, m * PW:(m + 1) * PW] = pltpu.bitcast(stage[slot, m].T, u32)
            wo_vm[j] = pltpu.bitcast(stage[slot, 3], u32)

        def project_ahead(j, rows):
            for m in range(3):
                pre[j, rows, m * PW:(m + 1) * PW] = _dot_nt(xsel[rows, :], stage[j % _RING, m])

        def plain_body(j, carry):
            @pl.when(j == 2)
            def _():
                for c in tile_copies(0):
                    c.start()

            fetch_pair(j)
            project_ahead(j, slice(None))
            repack_pair(j)
            return carry

        jax.lax.fori_loop(0, n_plain, plain_body, 0)

        def conv_body(c, carry):
            @pl.when(c + 1 < n_ct)
            def _():
                for copy in tile_copies(c + 1):
                    copy.start()

            @pl.when(c + 1 == n_ct)
            def _():
                x_copy.start()

            for copy in tile_copies(c):
                copy.wait()
            cols = pl.ds(pl.multiple_of(c * 128, 128), 128)
            fwd = fwd_ref[...]
            prev = None
            for a in range(n_blk):
                cur = _dot_nt(fwd, g_vm[c, :, pl.ds(a * _BLK, _BLK)])
                if prev is None:
                    g_hat[a] = cur
                else:
                    g_hat[a, 0:half, :] = cur[0:half] - prev[_BLK:_BLK + half]
                    g_hat[a, half:_BLK, :] = cur[half:_BLK] + prev[_BLK + half:]
                    g_hat[a, _BLK:_BLK + half, :] = cur[_BLK:_BLK + half] + prev[0:half]
                    g_hat[a, _BLK + half:, :] = cur[_BLK + half:] - prev[half:_BLK]
                prev = cur
            kpad[8:8 + S, :] = k_vm[c].astype(f32)
            sh = shift_ref[:, cols].astype(f32)
            for a in range(n_blk):
                rows = pl.ds(a * _BLK, _BLK)
                acc = kpad[pl.ds(8 + a * _BLK, _BLK), :] * sh[0:1, :]
                for i in range(1, ks):
                    acc = acc + kpad[pl.ds(8 + a * _BLK - i, _BLK), :] * sh[i:i + 1, :]
                kv = acc * v_vm[c, rows, :].astype(f32)
                kv_vm[rows, :] = kv
                u_hat[a] = _dot(fwd, kv.astype(bf16))

            def product_body(i, carry2):
                j = n_plain + 2 * c + i
                fetch_pair(j)
                n_rows = n_seg * _PRE
                pace = []
                for m in range(3):
                    total = None
                    for kt in range(n_ct):
                        kk = slice(kt * 128, (kt + 1) * 128)
                        t = _dot_nt(xsel[:, kk], stage[j % _RING, m, :, kk])
                        pace += [t[q:q + 8, 0:128] for q in range(0, n_rows, 8)]
                        total = t if total is None else total + t
                    pre[j, :, m * PW:(m + 1) * PW] = total
                repack_pair(j)
                n_freq = _BLK // 2
                n_mac = (n_freq // 8) * n_blk * (n_blk + 1) // 2
                done = 0
                for r in range(0, n_freq, 8):
                    re = pl.ds(pl.multiple_of(i * n_freq + r, 8), 8)
                    im = pl.ds(pl.multiple_of(i * n_freq + r + _BLK, 8), 8)
                    for a in range(n_blk):
                        yr = yi = None
                        for b in range(a + 1):
                            gr, gi = g_hat[b, re, :], g_hat[b, im, :]
                            ur, ui = u_hat[a - b, re, :], u_hat[a - b, im, :]
                            if b % 4 == 0:
                                gr = jnp.where(i < 0, pace[done * len(pace) // n_mac], gr)
                            tr, ti = gr * ur - gi * ui, gr * ui + gi * ur
                            yr = tr if yr is None else yr + tr
                            yi = ti if yi is None else yi + ti
                            done += 1
                        y_hat[a, re, :] = yr
                        y_hat[a, im, :] = yi
                return carry2

            jax.lax.fori_loop(0, 2, product_body, 0)

            inv = inv_ref[...]
            dsk = skip_vm[:, cols]
            for a in range(n_blk):
                rows = pl.ds(a * _BLK, _BLK)
                y_vm[rows, cols] = _dot(inv, y_hat[a].astype(bf16)) + kv_vm[rows, :] * dsk
            return carry

        jax.lax.fori_loop(0, n_ct, conv_body, 0)
        x_copy.wait()

        row = jax.lax.broadcasted_iota(jnp.int32, (L, 2 * L), 0)
        col = jax.lax.broadcasted_iota(jnp.int32, (L, 2 * L), 1)
        first = col < L
        visible = (row < M) | (row >= jnp.where(first, col, col - L))
        lane_first = jax.lax.broadcasted_iota(jnp.int32, (L, PW), 1) < Dh
        gw = gw_ref[...].astype(f32).reshape(1, D)

        def stack(t):
            zero = jnp.zeros_like(t)
            both = jnp.concatenate(
                [jnp.where(lane_first, t, zero), jnp.where(lane_first, zero, t)], axis=0)
            return both.astype(bf16)

        def step(s, mem):
            xs = x_vm[s].astype(f32)
            h = jnp.concatenate([mem, xs[0:seg - _PRE]], axis=0)
            ahead = pl.ds(pl.multiple_of(s * _PRE, _PRE), _PRE)
            qkv, p, o = {}, {}, {}
            acc = None
            for op, j in _step_schedule(n_pair):
                if op == "P":
                    qkv[j] = jnp.concatenate(
                        [_dot(h, pltpu.bitcast(wqkv[j], bf16)), pre[j, ahead, :]], axis=0)
                elif op == "S":
                    sc = _dot_nt(qkv[j][:, 0:PW], stack(qkv[j][:, PW:2 * PW])) * scale
                    sc = jnp.where(visible, sc, -1e9)
                    m0 = jnp.max(jnp.where(first, sc, -jnp.inf), axis=-1, keepdims=True)
                    m1 = jnp.max(jnp.where(first, -jnp.inf, sc), axis=-1, keepdims=True)
                    e = jnp.exp(sc - jnp.where(first, m0, m1))
                    s0 = jnp.sum(jnp.where(first, e, 0.0), axis=-1, keepdims=True)
                    s1 = jnp.sum(jnp.where(first, 0.0, e), axis=-1, keepdims=True)
                    p[j] = e / jnp.where(first, s0, s1)
                elif op == "V":
                    o[j] = _dot(p[j], stack(qkv[j][:, 2 * PW:]))
                else:
                    t = _dot(o[j], pltpu.bitcast(wo_vm[j], bf16))
                    acc = t if acc is None else acc + t
            gate = jax.nn.sigmoid(jnp.sum(xs * gw, axis=-1, keepdims=True))
            b = xs * y_vm[pl.ds(pl.multiple_of(s * seg, seg), seg), :]
            out_vm[s] = (gate * acc[M:] + (1.0 - gate) * b).astype(bf16)
            return acc[0:M]

        def out_copy(i):
            segs = pl.ds(i * _UNROLL, _UNROLL)
            return pltpu.make_async_copy(out_vm.at[segs], out_hbm.at[segs], out_sem)

        def steps(i, mem):
            for u in range(_UNROLL):
                mem = step(i * _UNROLL + u, mem)
            out_copy(i).start()
            return mem

        jax.lax.fori_loop(0, n_seg // _UNROLL, steps, mem0_ref[...].astype(f32))
        pltpu.make_async_copy(out_vm, out_hbm, out_sem).wait()

    return kernel


def pallas_gated_mix__memory_aug_recurrent_mem_tr__ssm_conv_h3__prompt_kernel(
    A_x, A_mem0, A_Wq, A_Wk, A_Wv, A_Wo, A_seg_len, B_q, B_k, B_v,
    B_shift_k, B_ssm_k, B_ssm_D, gate_w,
):
    del B_q
    seg = int(A_seg_len)
    B, S, D = A_x.shape
    _, H, Dh = A_Wq.shape
    M = A_mem0.shape[1]
    ks = B_shift_k.shape[1]
    PW = 2 * Dh
    n_pair = H // 2
    n_blk = S // _BLK
    n_seg = S // seg
    assert B == 1 and H % 2 == 0 and PW % 128 == 0 and D % 128 == 0
    assert S % _BLK == 0 and S % (_UNROLL * seg) == 0 and seg % 16 == 0
    assert M % 8 == 0 and ks <= 8 and n_pair >= 2 * (D // 128) + 5
    f32, bf16, u32 = jnp.float32, jnp.bfloat16, jnp.uint32
    fwd, inv = _dft_matrices()

    def heads_major(w):
        return jnp.transpose(w, (1, 2, 0)).reshape(H * Dh, D)

    hbm = pl.BlockSpec(memory_space=pl.ANY)
    vmem = pl.BlockSpec(memory_space=pltpu.VMEM)
    out = pl.pallas_call(
        _make_kernel(S, D, H, Dh, M, seg, ks),
        out_shape=jax.ShapeDtypeStruct((n_seg, seg, D), A_x.dtype),
        in_specs=[hbm, vmem, hbm, hbm, hbm, hbm, hbm, hbm,
                  vmem, hbm, vmem, vmem, vmem, vmem],
        out_specs=hbm,
        scratch_shapes=[
            pltpu.VMEM((n_seg, seg, D), bf16),
            pltpu.VMEM((n_seg, _PRE, D), bf16),
            pltpu.VMEM((n_seg * _PRE, D), bf16),
            pltpu.VMEM((D // 128, S, 128), bf16),
            pltpu.VMEM((D // 128, S, 128), bf16),
            pltpu.VMEM((D // 128, 128, S), bf16),
            pltpu.VMEM((_RING, 4, PW, D), bf16),
            pltpu.VMEM((n_pair, D // 2, 3 * PW), u32),
            pltpu.VMEM((n_pair, PW // 2, D), u32),
            pltpu.VMEM((n_pair, n_seg * _PRE, 3 * PW), f32),
            pltpu.VMEM((1, D), f32),
            pltpu.VMEM((S + 8, 128), f32),
            pltpu.VMEM((S, 128), f32),
            pltpu.VMEM((n_blk, 2 * _BLK, 128), f32),
            pltpu.VMEM((n_blk, 2 * _BLK, 128), f32),
            pltpu.VMEM((n_blk, 2 * _BLK, 128), f32),
            pltpu.VMEM((S, D), f32),
            pltpu.VMEM((n_seg, seg, D), bf16),
            pltpu.SemaphoreType.DMA((2,)),
            pltpu.SemaphoreType.DMA((D // 128,)),
            pltpu.SemaphoreType.DMA((_RING * 4,)),
            pltpu.SemaphoreType.DMA(()),
        ],
        compiler_params=pltpu.CompilerParams(vmem_limit_bytes=120 * 1024 * 1024),
    )(
        A_x.reshape(n_seg, seg, D), A_mem0.reshape(M, D),
        heads_major(A_Wq), heads_major(A_Wk), heads_major(A_Wv),
        A_Wo.reshape(H * Dh, D), B_k.reshape(S, D), B_v.reshape(S, D),
        B_shift_k.T, B_ssm_k, B_ssm_D, gate_w,
        jnp.asarray(fwd, bf16), jnp.asarray(inv, bf16),
    )
    return out.reshape(B, S, D)
```

```python
import numpy as np

import jax
import jax.numpy as jnp
import jax.experimental.pallas as pl
import jax.experimental.pallas.tpu as pltpu

_BLK = 128
_RING = 4
_PRE = 8
_ORDER, _LAG, _TAIL = "POVS", dict(S=1, V=3, O=9), "OOVSOOVOOOV"
_UNROLL = 4


def _dft_matrices():
    f = np.concatenate([np.arange(0, _BLK, 2), np.arange(1, _BLK, 2)])
    t = np.arange(_BLK)
    ang = 2.0 * np.pi * (f[:, None] + 0.5) * t[None, :] / (2 * _BLK)
    fwd = np.concatenate([np.cos(ang), -np.sin(ang)], axis=0)
    inv = fwd.T / _BLK
    return fwd.astype(np.float32), inv.astype(np.float32)


def _dot(a, b):
    return jax.lax.dot_general(
        a, b, (((1,), (0,)), ((), ())), preferred_element_type=jnp.float32)


def _dot_nt(a, b):
    return jax.lax.dot_general(
        a, b, (((1,), (1,)), ((), ())), preferred_element_type=jnp.float32)


def _step_schedule(n):
    lag = dict(P=0, **_LAG)
    done = dict.fromkeys("PSVO", 0)
    sched = []

    def emit(op):
        if done[op] < n:
            sched.append((op, done[op]))
            done[op] += 1

    for j in range(n):
        for op in _ORDER:
            if j >= lag[op]:
                emit(op)
    for op in _TAIL:
        emit(op)
    while done["O"] < n:
        emit("O")
    return sched


def _make_kernel(S, D, H, Dh, M, seg, ks):
    L = M + seg
    n_seg = S // seg
    n_pair = H // 2
    PW = 2 * Dh
    n_blk = S // _BLK
    n_ct = D // 128
    n_plain = n_pair - 2 * n_ct
    half = _BLK // 2
    spec = slice(0, 2 * _BLK)
    scale = float(Dh) ** -0.5
    f32, bf16, u32 = jnp.float32, jnp.bfloat16, jnp.uint32

    def kernel(x_hbm, mem0_ref, wq_hbm, wk_hbm, wv_hbm, wo_hbm, k_hbm, v_hbm,
               shift_ref, g_hbm, dskip_ref, gw_ref, fwd_ref, inv_ref,
               out_hbm,
               x_vm, xs_vm, xsel, k_vm, v_vm, g_vm, stage, wqkv, wo_vm, pre,
               skip_vm, kpad, kv_vm, u_hat, g_hat, y_hat, y_vm, out_vm,
               in_sem, tile_sem, w_sem, out_sem):
        xs_copy = pltpu.make_async_copy(
            x_hbm.at[:, pl.ds(seg - _PRE, _PRE), :], xs_vm, in_sem.at[0])
        x_copy = pltpu.make_async_copy(x_hbm, x_vm, in_sem.at[1])

        def tile_copies(c):
            cols = pl.ds(pl.multiple_of(c * 128, 128), 128)
            return [
                pltpu.make_async_copy(g_hbm.at[cols, :], g_vm.at[c], tile_sem.at[c]),
                pltpu.make_async_copy(k_hbm.at[:, cols], k_vm.at[c], tile_sem.at[c]),
                pltpu.make_async_copy(v_hbm.at[:, cols], v_vm.at[c], tile_sem.at[c]),
            ]

        def w_copies(j):
            slot = j % _RING
            rows = pl.ds(pl.multiple_of(j * PW, PW), PW)
            return [
                pltpu.make_async_copy(
                    src.at[rows, :], stage.at[slot, m], w_sem.at[slot * 4 + m])
                for m, src in enumerate((wq_hbm, wk_hbm, wv_hbm, wo_hbm))]

        xs_copy.start()
        for c in w_copies(0):
            c.start()
        xs_copy.wait()
        for j in range(1, _RING - 1):
            for c in w_copies(j):
                c.start()
        xsel[...] = xs_vm[...].astype(f32).reshape(n_seg * _PRE, D).astype(bf16)
        kpad[0:8, :] = jnp.zeros((8, 128), f32)
        skip_vm[...] = dskip_ref[...].astype(f32).reshape(1, D)

        def fetch_pair(j):
            @pl.when(j + _RING - 1 < n_pair)
            def _():
                for c in w_copies(j + _RING - 1):
                    c.start()

            for c in w_copies(j):
                c.wait()

        def repack_pair(j):
            slot = j % _RING
            for m in range(3):
                wqkv[j, :, m * PW:(m + 1) * PW] = pltpu.bitcast(stage[slot, m].T, u32)
            wo_vm[j] = pltpu.bitcast(stage[slot, 3], u32)

        def project_ahead(j, rows):
            for m in range(3):
                pre[j, rows, m * PW:(m + 1) * PW] = _dot_nt(xsel[rows, :], stage[j % _RING, m])

        def plain_body(j, carry):
            @pl.when(j == 2)
            def _():
                for c in tile_copies(0):
                    c.start()

            fetch_pair(j)
            project_ahead(j, slice(None))
            repack_pair(j)
            return carry

        jax.lax.fori_loop(0, n_plain, plain_body, 0)

        def conv_body(c, carry):
            @pl.when(c + 1 < n_ct)
            def _():
                for copy in tile_copies(c + 1):
                    copy.start()

            @pl.when(c + 1 == n_ct)
            def _():
                x_copy.start()

            for copy in tile_copies(c):
                copy.wait()
            cols = pl.ds(pl.multiple_of(c * 128, 128), 128)
            fwd = fwd_ref[...]
            prev = None
            for a in range(n_blk):
                cur = _dot_nt(fwd, g_vm[c, :, pl.ds(a * _BLK, _BLK)])
                if prev is None:
                    g_hat[a, spec, :] = cur
                else:
                    g_hat[a, 0:half, :] = cur[0:half] - prev[_BLK:_BLK + half]
                    g_hat[a, half:_BLK, :] = cur[half:_BLK] + prev[_BLK + half:]
                    g_hat[a, _BLK:_BLK + half, :] = cur[_BLK:_BLK + half] + prev[0:half]
                    g_hat[a, _BLK + half:2 * _BLK, :] = cur[_BLK + half:] - prev[half:_BLK]
                prev = cur
            kpad[8:8 + S, :] = k_vm[c].astype(f32)
            sh = shift_ref[:, cols].astype(f32)
            for a in range(n_blk):
                rows = pl.ds(a * _BLK, _BLK)
                acc = kpad[pl.ds(8 + a * _BLK, _BLK), :] * sh[0:1, :]
                for i in range(1, ks):
                    acc = acc + kpad[pl.ds(8 + a * _BLK - i, _BLK), :] * sh[i:i + 1, :]
                kv = acc * v_vm[c, rows, :].astype(f32)
                kv_vm[rows, :] = kv
                u_hat[a, spec, :] = _dot(fwd, kv.astype(bf16))

            def product_body(i, carry2):
                j = n_plain + 2 * c + i
                fetch_pair(j)
                n_rows = n_seg * _PRE
                pace = []
                for m in range(3):
                    total = None
                    for kt in range(n_ct):
                        kk = slice(kt * 128, (kt + 1) * 128)
                        t = _dot_nt(xsel[:, kk], stage[j % _RING, m, :, kk])
                        pace += [t[q:q + 8, 0:128] for q in range(0, n_rows, 8)]
                        total = t if total is None else total + t
                    pre[j, :, m * PW:(m + 1) * PW] = total
                repack_pair(j)
                n_freq = _BLK // 2
                n_mac = (n_freq // 8) * n_blk * (n_blk + 1) // 2
                done = 0
                for r in range(0, n_freq, 8):
                    re = pl.ds(pl.multiple_of(i * n_freq + r, 8), 8)
                    im = pl.ds(pl.multiple_of(i * n_freq + r + _BLK, 8), 8)
                    for a0 in range(0, n_blk, 2):
                        yr, yi = {}, {}
                        for b in range(a0 + 2):
                            gr, gi = g_hat[b, re, :], g_hat[b, im, :]
                            if b % 2 == 0:
                                gr = jnp.where(i < 0, pace[done * len(pace) // n_mac], gr)
                            for a in range(max(b, a0), a0 + 2):
                                ur, ui = u_hat[a - b, re, :], u_hat[a - b, im, :]
                                tr, ti = gr * ur - gi * ui, gr * ui + gi * ur
                                yr[a] = yr[a] + tr if a in yr else tr
                                yi[a] = yi[a] + ti if a in yi else ti
                                done += 1
                        for a in yr:
                            y_hat[a, re, :] = yr[a]
                            y_hat[a, im, :] = yi[a]
                return carry2

            jax.lax.fori_loop(0, 2, product_body, 0)

            inv = inv_ref[...]
            dsk = skip_vm[:, cols]
            for a in range(n_blk):
                rows = pl.ds(a * _BLK, _BLK)
                y_vm[rows, cols] = _dot(inv, y_hat[a, spec, :].astype(bf16)) + kv_vm[rows, :] * dsk
            return carry

        jax.lax.fori_loop(0, n_ct, conv_body, 0)
        x_copy.wait()

        row = jax.lax.broadcasted_iota(jnp.int32, (L, 2 * L), 0)
        col = jax.lax.broadcasted_iota(jnp.int32, (L, 2 * L), 1)
        first = col < L
        visible = (row < M) | (row >= jnp.where(first, col, col - L))
        lane_first = jax.lax.broadcasted_iota(jnp.int32, (L, PW), 1) < Dh
        gw = gw_ref[...].astype(f32).reshape(1, D)

        def stack(t):
            zero = jnp.zeros_like(t)
            both = jnp.concatenate(
                [jnp.where(lane_first, t, zero), jnp.where(lane_first, zero, t)], axis=0)
            return both.astype(bf16)

        def step(s, mem):
            xs = x_vm[s].astype(f32)
            h = jnp.concatenate([mem, xs[0:seg - _PRE]], axis=0)
            ahead = pl.ds(pl.multiple_of(s * _PRE, _PRE), _PRE)
            qkv, p, o = {}, {}, {}
            acc = None
            for op, j in _step_schedule(n_pair):
                if op == "P":
                    qkv[j] = jnp.concatenate(
                        [_dot(h, pltpu.bitcast(wqkv[j], bf16)), pre[j, ahead, :]], axis=0)
                elif op == "S":
                    sc = _dot_nt(qkv[j][:, 0:PW], stack(qkv[j][:, PW:2 * PW])) * scale
                    sc = jnp.where(visible, sc, -1e9)
                    m0 = jnp.max(jnp.where(first, sc, -jnp.inf), axis=-1, keepdims=True)
                    m1 = jnp.max(jnp.where(first, -jnp.inf, sc), axis=-1, keepdims=True)
                    e = jnp.exp(sc - jnp.where(first, m0, m1))
                    s0 = jnp.sum(jnp.where(first, e, 0.0), axis=-1, keepdims=True)
                    s1 = jnp.sum(jnp.where(first, 0.0, e), axis=-1, keepdims=True)
                    p[j] = e / jnp.where(first, s0, s1)
                elif op == "V":
                    o[j] = _dot(p[j], stack(qkv[j][:, 2 * PW:]))
                else:
                    t = _dot(o[j], pltpu.bitcast(wo_vm[j], bf16))
                    acc = t if acc is None else acc + t
            gate = jax.nn.sigmoid(jnp.sum(xs * gw, axis=-1, keepdims=True))
            b = xs * y_vm[pl.ds(pl.multiple_of(s * seg, seg), seg), :]
            out_vm[s] = (gate * acc[M:] + (1.0 - gate) * b).astype(bf16)
            return acc[0:M]

        def out_copy(i):
            segs = pl.ds(i * _UNROLL, _UNROLL)
            return pltpu.make_async_copy(out_vm.at[segs], out_hbm.at[segs], out_sem)

        def steps(i, mem):
            for u in range(_UNROLL):
                mem = step(i * _UNROLL + u, mem)
            out_copy(i).start()
            return mem

        jax.lax.fori_loop(0, n_seg // _UNROLL, steps, mem0_ref[...].astype(f32))
        pltpu.make_async_copy(out_vm, out_hbm, out_sem).wait()

    return kernel


def pallas_gated_mix__memory_aug_recurrent_mem_tr__ssm_conv_h3__prompt_kernel(
    A_x, A_mem0, A_Wq, A_Wk, A_Wv, A_Wo, A_seg_len, B_q, B_k, B_v,
    B_shift_k, B_ssm_k, B_ssm_D, gate_w,
):
    del B_q
    seg = int(A_seg_len)
    B, S, D = A_x.shape
    _, H, Dh = A_Wq.shape
    M = A_mem0.shape[1]
    ks = B_shift_k.shape[1]
    PW = 2 * Dh
    n_pair = H // 2
    n_blk = S // _BLK
    n_seg = S // seg
    assert B == 1 and H % 2 == 0 and PW % 128 == 0 and D % 128 == 0
    assert S % _BLK == 0 and S % (_UNROLL * seg) == 0 and seg % 16 == 0
    assert M % 8 == 0 and ks <= 8 and n_pair >= 2 * (D // 128) + 5
    f32, bf16, u32 = jnp.float32, jnp.bfloat16, jnp.uint32
    fwd, inv = _dft_matrices()

    def heads_major(w):
        return jnp.transpose(w, (1, 2, 0)).reshape(H * Dh, D)

    hbm = pl.BlockSpec(memory_space=pl.ANY)
    vmem = pl.BlockSpec(memory_space=pltpu.VMEM)
    out = pl.pallas_call(
        _make_kernel(S, D, H, Dh, M, seg, ks),
        out_shape=jax.ShapeDtypeStruct((n_seg, seg, D), A_x.dtype),
        in_specs=[hbm, vmem, hbm, hbm, hbm, hbm, hbm, hbm,
                  vmem, hbm, vmem, vmem, vmem, vmem],
        out_specs=hbm,
        scratch_shapes=[
            pltpu.VMEM((n_seg, seg, D), bf16),
            pltpu.VMEM((n_seg, _PRE, D), bf16),
            pltpu.VMEM((n_seg * _PRE, D), bf16),
            pltpu.VMEM((D // 128, S, 128), bf16),
            pltpu.VMEM((D // 128, S, 128), bf16),
            pltpu.VMEM((D // 128, 128, S), bf16),
            pltpu.VMEM((_RING, 4, PW, D), bf16),
            pltpu.VMEM((n_pair, D // 2, 3 * PW), u32),
            pltpu.VMEM((n_pair, PW // 2, D), u32),
            pltpu.VMEM((n_pair, n_seg * _PRE, 3 * PW), f32),
            pltpu.VMEM((1, D), f32),
            pltpu.VMEM((S + 8, 128), f32),
            pltpu.VMEM((S, 128), f32),
            pltpu.VMEM((n_blk, 2 * _BLK + 24, 128), f32),
            pltpu.VMEM((n_blk, 2 * _BLK + 40, 128), f32),
            pltpu.VMEM((n_blk, 2 * _BLK + 8, 128), f32),
            pltpu.VMEM((S, D), f32),
            pltpu.VMEM((n_seg, seg, D), bf16),
            pltpu.SemaphoreType.DMA((2,)),
            pltpu.SemaphoreType.DMA((D // 128,)),
            pltpu.SemaphoreType.DMA((_RING * 4,)),
            pltpu.SemaphoreType.DMA(()),
        ],
        compiler_params=pltpu.CompilerParams(vmem_limit_bytes=120 * 1024 * 1024),
    )(
        A_x.reshape(n_seg, seg, D), A_mem0.reshape(M, D),
        heads_major(A_Wq), heads_major(A_Wk), heads_major(A_Wv),
        A_Wo.reshape(H * Dh, D), B_k.reshape(S, D), B_v.reshape(S, D),
        B_shift_k.T, B_ssm_k, B_ssm_D, gate_w,
        jnp.asarray(fwd, bf16), jnp.asarray(inv, bf16),
    )
    return out.reshape(B, S, D)
```

```python
import numpy as np

import jax
import jax.numpy as jnp
import jax.experimental.pallas as pl
import jax.experimental.pallas.tpu as pltpu

_BLK = 128
_RING = 4
_PRE = 8
_ORDER, _LAG, _TAIL = "POVS", dict(S=1, V=3, O=9), "OOVSOOVOOOVOOF"


def _dft_matrices():
    f = np.concatenate([np.arange(0, _BLK, 2), np.arange(1, _BLK, 2)])
    t = np.arange(_BLK)
    ang = 2.0 * np.pi * (f[:, None] + 0.5) * t[None, :] / (2 * _BLK)
    fwd = np.concatenate([np.cos(ang), -np.sin(ang)], axis=0)
    inv = fwd.reshape(2, _BLK // 8, 8, _BLK).transpose(3, 1, 0, 2).reshape(_BLK, 2 * _BLK)
    inv = inv / _BLK
    return fwd.astype(np.float32), inv.astype(np.float32)


def _dot(a, b):
    return jax.lax.dot_general(
        a, b, (((1,), (0,)), ((), ())), preferred_element_type=jnp.float32)


def _dot_nt(a, b):
    return jax.lax.dot_general(
        a, b, (((1,), (1,)), ((), ())), preferred_element_type=jnp.float32)


def _step_schedule(n):
    lag = dict(P=0, **_LAG)
    done = dict.fromkeys("PSVOF", 0)
    sched = []

    def emit(op):
        if done[op] < n:
            sched.append((op, done[op]))
            done[op] += 1

    for j in range(n):
        for op in _ORDER:
            if j >= lag[op]:
                emit(op)
    for op in _TAIL:
        emit(op)
    assert all(done[op] == n for op in "PSVO") and done["F"] == 1
    return sched


def _make_kernel(S, D, H, Dh, M, seg, ks):
    L = M + seg
    n_seg = S // seg
    n_pair = H // 2
    PW = 2 * Dh
    n_blk = S // _BLK
    n_ct = D // 128
    n_plain = n_pair - 2 * n_ct
    half = _BLK // 2
    per_blk = _BLK // seg
    spec = slice(0, 2 * _BLK)
    scale = float(Dh) ** -0.5
    f32, bf16, u32 = jnp.float32, jnp.bfloat16, jnp.uint32

    def kernel(x_hbm, mem0_ref, wq_hbm, wk_hbm, wv_hbm, wo_hbm, k_hbm, v_hbm,
               shift_ref, g_hbm, dskip_ref, gw_ref, fwd_ref, inv_ref,
               out_hbm,
               x_vm, xs_vm, xsel, k_vm, v_vm, g_vm, stage, wqkv, wo_vm, pre,
               dskip_vm, kpad, u_hat, g_hat, y_hat, skip, out_vm,
               in_sem, tile_sem, w_sem, out_sem):
        xs_copy = pltpu.make_async_copy(
            x_hbm.at[:, pl.ds(seg - _PRE, _PRE), :], xs_vm, in_sem.at[0])
        x_copy = pltpu.make_async_copy(x_hbm, x_vm, in_sem.at[1])

        def tile_copies(c):
            cols = pl.ds(pl.multiple_of(c * 128, 128), 128)
            return [
                pltpu.make_async_copy(g_hbm.at[cols, :], g_vm.at[c], tile_sem.at[c]),
                pltpu.make_async_copy(k_hbm.at[:, cols], k_vm.at[c], tile_sem.at[c]),
                pltpu.make_async_copy(v_hbm.at[:, cols], v_vm.at[c], tile_sem.at[c]),
            ]

        def w_copies(j):
            slot = j % _RING
            rows = pl.ds(pl.multiple_of(j * PW, PW), PW)
            return [
                pltpu.make_async_copy(
                    src.at[rows, :], stage.at[slot, m], w_sem.at[slot * 4 + m])
                for m, src in enumerate((wq_hbm, wk_hbm, wv_hbm, wo_hbm))]

        xs_copy.start()
        for c in w_copies(0):
            c.start()
        xs_copy.wait()
        for j in range(1, _RING - 1):
            for c in w_copies(j):
                c.start()
        xsel[...] = xs_vm[...].astype(f32).reshape(n_seg * _PRE, D).astype(bf16)
        kpad[0:8, :] = jnp.zeros((8, 128), f32)
        dskip_vm[...] = dskip_ref[...].astype(f32).reshape(1, D)

        def fetch_pair(j):
            @pl.when(j + _RING - 1 < n_pair)
            def _():
                for c in w_copies(j + _RING - 1):
                    c.start()

            for c in w_copies(j):
                c.wait()

        def repack_pair(j):
            slot = j % _RING
            for m in range(3):
                wqkv[j, :, m * PW:(m + 1) * PW] = pltpu.bitcast(stage[slot, m].T, u32)
            wo_vm[j] = pltpu.bitcast(stage[slot, 3], u32)

        def project_ahead(j, rows):
            for m in range(3):
                pre[j, rows, m * PW:(m + 1) * PW] = _dot_nt(xsel[rows, :], stage[j % _RING, m])

        def plain_body(j, carry):
            @pl.when(j == 2)
            def _():
                for c in tile_copies(0):
                    c.start()

            fetch_pair(j)
            project_ahead(j, slice(None))
            repack_pair(j)
            return carry

        jax.lax.fori_loop(0, n_plain, plain_body, 0)

        def conv_body(c, carry):
            @pl.when(c + 1 < n_ct)
            def _():
                for copy in tile_copies(c + 1):
                    copy.start()

            @pl.when(c + 1 == n_ct)
            def _():
                x_copy.start()

            for copy in tile_copies(c):
                copy.wait()
            cols = pl.ds(pl.multiple_of(c * 128, 128), 128)
            fwd = fwd_ref[...]
            prev = None
            for a in range(n_blk):
                cur = _dot_nt(fwd, g_vm[c, :, pl.ds(a * _BLK, _BLK)])
                if prev is None:
                    g_hat[a, spec, :] = cur
                else:
                    g_hat[a, 0:half, :] = cur[0:half] - prev[_BLK:_BLK + half]
                    g_hat[a, half:_BLK, :] = cur[half:_BLK] + prev[_BLK + half:]
                    g_hat[a, _BLK:_BLK + half, :] = cur[_BLK:_BLK + half] + prev[0:half]
                    g_hat[a, _BLK + half:2 * _BLK, :] = cur[_BLK + half:] - prev[half:_BLK]
                prev = cur
            kpad[8:8 + S, :] = k_vm[c].astype(f32)
            sh = shift_ref[:, cols].astype(f32)
            dsk = dskip_vm[:, cols]
            for a in range(n_blk):
                rows = pl.ds(a * _BLK, _BLK)
                acc = kpad[pl.ds(8 + a * _BLK, _BLK), :] * sh[0:1, :]
                for i in range(1, ks):
                    acc = acc + kpad[pl.ds(8 + a * _BLK - i, _BLK), :] * sh[i:i + 1, :]
                kv = acc * v_vm[c, rows, :].astype(f32)
                skip[rows, cols] = kv * dsk
                u_hat[a, spec, :] = _dot(fwd, kv.astype(bf16))

            def product_body(i, carry2):
                j = n_plain + 2 * c + i
                fetch_pair(j)
                n_rows = n_seg * _PRE
                pace = []
                for m in range(3):
                    total = None
                    for kt in range(n_ct):
                        kk = slice(kt * 128, (kt + 1) * 128)
                        t = _dot_nt(xsel[:, kk], stage[j % _RING, m, :, kk])
                        pace += [t[q:q + 8, 0:128] for q in range(0, n_rows, 8)]
                        total = t if total is None else total + t
                    pre[j, :, m * PW:(m + 1) * PW] = total
                repack_pair(j)
                n_freq = _BLK // 2
                n_mac = (n_freq // 8) * n_blk * (n_blk + 1) // 2
                done = 0
                for r in range(0, n_freq, 8):
                    re = pl.ds(pl.multiple_of(i * n_freq + r, 8), 8)
                    im = pl.ds(pl.multiple_of(i * n_freq + r + _BLK, 8), 8)
                    for a0 in range(0, n_blk, 2):
                        yr, yi = {}, {}
                        for b in range(a0 + 2):
                            gr, gi = g_hat[b, re, :], g_hat[b, im, :]
                            if b % 2 == 0:
                                gr = jnp.where(i < 0, pace[done * len(pace) // n_mac], gr)
                            for a in range(max(b, a0), a0 + 2):
                                ur, ui = u_hat[a - b, re, :], u_hat[a - b, im, :]
                                tr, ti = gr * ur - gi * ui, gr * ui + gi * ur
                                yr[a] = yr[a] + tr if a in yr else tr
                                yi[a] = yi[a] + ti if a in yi else ti
                                done += 1
                        for a in yr:
                            y = jnp.concatenate([yr[a], yi[a]], axis=0).astype(bf16)
                            y_hat[a, re, cols] = pltpu.bitcast(y, u32)
                return carry2

            jax.lax.fori_loop(0, 2, product_body, 0)
            return carry

        jax.lax.fori_loop(0, n_ct, conv_body, 0)
        x_copy.wait()

        row = jax.lax.broadcasted_iota(jnp.int32, (L, 2 * L), 0)
        col = jax.lax.broadcasted_iota(jnp.int32, (L, 2 * L), 1)
        first = col < L
        visible = (row < M) | (row >= jnp.where(first, col, col - L))
        lane_first = jax.lax.broadcasted_iota(jnp.int32, (L, PW), 1) < Dh
        gw = gw_ref[...].astype(f32).reshape(1, D)

        def stack(t):
            zero = jnp.zeros_like(t)
            both = jnp.concatenate(
                [jnp.where(lane_first, t, zero), jnp.where(lane_first, zero, t)], axis=0)
            return both.astype(bf16)

        def step(blk, part, mem):
            s = blk * per_blk + part
            xs = x_vm[s].astype(f32)
            h = jnp.concatenate([mem, xs[0:seg - _PRE]], axis=0)
            ahead = pl.ds(pl.multiple_of(s * _PRE, _PRE), _PRE)
            qkv, p, o = {}, {}, {}
            acc = None
            for op, j in _step_schedule(n_pair):
                if op == "P":
                    qkv[j] = jnp.concatenate(
                        [_dot(h, pltpu.bitcast(wqkv[j], bf16)), pre[j, ahead, :]], axis=0)
                elif op == "S":
                    sc = _dot_nt(qkv[j][:, 0:PW], stack(qkv[j][:, PW:2 * PW])) * scale
                    sc = jnp.where(visible, sc, -1e9)
                    m0 = jnp.max(jnp.where(first, sc, -jnp.inf), axis=-1, keepdims=True)
                    m1 = jnp.max(jnp.where(first, -jnp.inf, sc), axis=-1, keepdims=True)
                    e = jnp.exp(sc - jnp.where(first, m0, m1))
                    s0 = jnp.sum(jnp.where(first, e, 0.0), axis=-1, keepdims=True)
                    s1 = jnp.sum(jnp.where(first, 0.0, e), axis=-1, keepdims=True)
                    p[j] = e / jnp.where(first, s0, s1)
                elif op == "V":
                    o[j] = _dot(p[j], stack(qkv[j][:, 2 * PW:]))
                elif op == "O":
                    t = _dot(o[j], pltpu.bitcast(wo_vm[j], bf16))
                    acc = t if acc is None else acc + t
                else:
                    y = _dot(inv_ref[part * seg:(part + 1) * seg, :],
                             pltpu.bitcast(y_hat[blk], bf16))
            b = xs * (y + skip[pl.ds(pl.multiple_of(s * seg, seg), seg), :])
            gate = jax.nn.sigmoid(jnp.sum(xs * gw, axis=-1, keepdims=True))
            out_vm[s] = (gate * acc[M:] + (1.0 - gate) * b).astype(bf16)
            return acc[0:M]

        def steps(blk, mem):
            for part in range(per_blk):
                mem = step(blk, part, mem)
            segs = pl.ds(blk * per_blk, per_blk)
            pltpu.make_async_copy(out_vm.at[segs], out_hbm.at[segs], out_sem).start()
            return mem

        jax.lax.fori_loop(0, n_blk, steps, mem0_ref[...].astype(f32))
        pltpu.make_async_copy(out_vm, out_hbm, out_sem).wait()

    return kernel


def pallas_gated_mix__memory_aug_recurrent_mem_tr__ssm_conv_h3__prompt_kernel(
    A_x, A_mem0, A_Wq, A_Wk, A_Wv, A_Wo, A_seg_len, B_q, B_k, B_v,
    B_shift_k, B_ssm_k, B_ssm_D, gate_w,
):
    del B_q
    seg = int(A_seg_len)
    B, S, D = A_x.shape
    _, H, Dh = A_Wq.shape
    M = A_mem0.shape[1]
    ks = B_shift_k.shape[1]
    PW = 2 * Dh
    n_pair = H // 2
    n_blk = S // _BLK
    n_seg = S // seg
    assert B == 1 and H % 2 == 0 and PW % 128 == 0 and D % 128 == 0
    assert S % _BLK == 0 and _BLK % seg == 0 and seg % 16 == 0
    assert M % 8 == 0 and ks <= 8 and n_pair >= 2 * (D // 128) + 5
    f32, bf16, u32 = jnp.float32, jnp.bfloat16, jnp.uint32
    fwd, inv = _dft_matrices()

    def heads_major(w):
        return jnp.transpose(w, (1, 2, 0)).reshape(H * Dh, D)

    hbm = pl.BlockSpec(memory_space=pl.ANY)
    vmem = pl.BlockSpec(memory_space=pltpu.VMEM)
    out = pl.pallas_call(
        _make_kernel(S, D, H, Dh, M, seg, ks),
        out_shape=jax.ShapeDtypeStruct((n_seg, seg, D), A_x.dtype),
        in_specs=[hbm, vmem, hbm, hbm, hbm, hbm, hbm, hbm,
                  vmem, hbm, vmem, vmem, vmem, vmem],
        out_specs=hbm,
        scratch_shapes=[
            pltpu.VMEM((n_seg, seg, D), bf16),
            pltpu.VMEM((n_seg, _PRE, D), bf16),
            pltpu.VMEM((n_seg * _PRE, D), bf16),
            pltpu.VMEM((D // 128, S, 128), bf16),
            pltpu.VMEM((D // 128, S, 128), bf16),
            pltpu.VMEM((D // 128, 128, S), bf16),
            pltpu.VMEM((_RING, 4, PW, D), bf16),
            pltpu.VMEM((n_pair, D // 2, 3 * PW), u32),
            pltpu.VMEM((n_pair, PW // 2, D), u32),
            pltpu.VMEM((n_pair, n_seg * _PRE, 3 * PW), f32),
            pltpu.VMEM((1, D), f32),
            pltpu.VMEM((S + 8, 128), f32),
            pltpu.VMEM((n_blk, 2 * _BLK + 24, 128), f32),
            pltpu.VMEM((n_blk, 2 * _BLK + 40, 128), f32),
            pltpu.VMEM((n_blk, _BLK, D), u32),
            pltpu.VMEM((S, D), f32),
            pltpu.VMEM((n_seg, seg, D), bf16),
            pltpu.SemaphoreType.DMA((2,)),
            pltpu.SemaphoreType.DMA((D // 128,)),
            pltpu.SemaphoreType.DMA((_RING * 4,)),
            pltpu.SemaphoreType.DMA(()),
        ],
        compiler_params=pltpu.CompilerParams(vmem_limit_bytes=120 * 1024 * 1024),
    )(
        A_x.reshape(n_seg, seg, D), A_mem0.reshape(M, D),
        heads_major(A_Wq), heads_major(A_Wk), heads_major(A_Wv),
        A_Wo.reshape(H * Dh, D), B_k.reshape(S, D), B_v.reshape(S, D),
        B_shift_k.T, B_ssm_k, B_ssm_D, gate_w,
        jnp.asarray(fwd, bf16), jnp.asarray(inv, bf16),
    )
    return out.reshape(B, S, D)
```

```python
import numpy as np

import jax
import jax.numpy as jnp
import jax.experimental.pallas as pl
import jax.experimental.pallas.tpu as pltpu

_BLK = 128
_PRE = 8
_ORDER, _LAG, _TAIL = "POVS", dict(S=1, V=3, O=9), "OOVSOOVOOOVOOF"


def _dft_matrices():
    f = np.concatenate([np.arange(0, _BLK, 2), np.arange(1, _BLK, 2)])
    t = np.arange(_BLK)
    ang = 2.0 * np.pi * (f[:, None] + 0.5) * t[None, :] / (2 * _BLK)
    fwd = np.concatenate([np.cos(ang), -np.sin(ang)], axis=0)
    inv = fwd.reshape(2, _BLK // 8, 8, _BLK).transpose(3, 1, 0, 2).reshape(_BLK, 2 * _BLK)
    inv = inv / _BLK
    return fwd.astype(np.float32), inv.astype(np.float32)


def _dot(a, b):
    return jax.lax.dot_general(
        a, b, (((1,), (0,)), ((), ())), preferred_element_type=jnp.float32)


def _dot_nt(a, b):
    return jax.lax.dot_general(
        a, b, (((1,), (1,)), ((), ())), preferred_element_type=jnp.float32)


def _step_schedule(n):
    lag = dict(P=0, **_LAG)
    done = dict.fromkeys("PSVOF", 0)
    sched = []

    def emit(op):
        if done[op] < n:
            sched.append((op, done[op]))
            done[op] += 1

    for j in range(n):
        for op in _ORDER:
            if j >= lag[op]:
                emit(op)
    for op in _TAIL:
        emit(op)
    assert all(done[op] == n for op in "PSVO") and done["F"] == 1
    return sched


def _make_kernel(S, D, H, Dh, M, seg, ks):
    L = M + seg
    n_seg = S // seg
    n_pair = H // 2
    PW = 2 * Dh
    n_blk = S // _BLK
    n_ct = D // 128
    n_plain = n_pair - 2 * n_ct
    half = _BLK // 2
    per_blk = _BLK // seg
    spec = slice(0, 2 * _BLK)
    scale = float(Dh) ** -0.5
    f32, bf16, u32 = jnp.float32, jnp.bfloat16, jnp.uint32

    def kernel(x_hbm, mem0_ref, wq_hbm, wk_hbm, wv_hbm, wo_hbm, k_hbm, v_hbm,
               shift_ref, g_hbm, dskip_ref, gw_ref, fwd_ref, inv_ref,
               out_hbm,
               x_vm, xs_vm, xsel, k_vm, v_vm, g_vm, stage, wqkv, wo_vm, pre,
               dskip_vm, kpad, u_hat, g_hat, y_hat, skip, out_vm,
               in_sem, tile_sem, w_sem, out_sem):
        xs_copy = pltpu.make_async_copy(
            x_hbm.at[:, pl.ds(seg - _PRE, _PRE), :], xs_vm, in_sem.at[0])
        x_copy = pltpu.make_async_copy(x_hbm, x_vm, in_sem.at[1])

        def tile_copies(c):
            cols = pl.ds(pl.multiple_of(c * 128, 128), 128)
            return [
                pltpu.make_async_copy(g_hbm.at[cols, :], g_vm.at[c], tile_sem.at[c]),
                pltpu.make_async_copy(k_hbm.at[:, cols], k_vm.at[c], tile_sem.at[c]),
                pltpu.make_async_copy(v_hbm.at[:, cols], v_vm.at[c], tile_sem.at[c]),
            ]

        def w_copies(j):
            slot = j % 2
            rows = pl.ds(pl.multiple_of(j * PW, PW), PW)
            return [
                pltpu.make_async_copy(
                    src.at[rows, :], stage.at[slot, m], w_sem.at[slot * 4 + m])
                for m, src in enumerate((wq_hbm, wk_hbm, wv_hbm, wo_hbm))]

        def fetch_pair(j):
            @pl.when(j + 1 < n_pair)
            def _():
                for c in w_copies(j + 1):
                    c.start()

            for c in w_copies(j):
                c.wait()

        def repack_pair(j):
            for m in range(3):
                wqkv[j, :, m * PW:(m + 1) * PW] = pltpu.bitcast(stage[j % 2, m].T, u32)
            wo_vm[j] = pltpu.bitcast(stage[j % 2, 3], u32)

        def project_ahead(j, m):
            pre[j, :, m * PW:(m + 1) * PW] = _dot_nt(xsel[...], stage[j % 2, m])

        first_copies = w_copies(0)
        xs_copy.start()
        first_copies[0].start()
        kpad[0:8, :] = jnp.zeros((8, 128), f32)
        dskip_vm[...] = dskip_ref[...].astype(f32).reshape(1, D)
        xs_copy.wait()
        first_copies[0].wait()
        for c in first_copies[1:3]:
            c.start()
        xsel[...] = xs_vm[...].astype(f32).reshape(n_seg * _PRE, D).astype(bf16)
        project_ahead(0, 0)
        for c in first_copies[1:3]:
            c.wait()
        for c in first_copies[3:] + w_copies(1):
            c.start()
        project_ahead(0, 1)
        project_ahead(0, 2)
        first_copies[3].wait()
        repack_pair(0)

        def plain_body(j, carry):
            for i, c in enumerate(tile_copies(0)):
                @pl.when(j == 1 + i)
                def _():
                    c.start()

            fetch_pair(j)
            for m in range(3):
                project_ahead(j, m)
            repack_pair(j)
            return carry

        jax.lax.fori_loop(1, n_plain, plain_body, 0)

        def conv_body(c, carry):
            @pl.when(c + 1 < n_ct)
            def _():
                for copy in tile_copies(c + 1):
                    copy.start()

            @pl.when(c + 1 == n_ct)
            def _():
                x_copy.start()

            for copy in tile_copies(c):
                copy.wait()
            cols = pl.ds(pl.multiple_of(c * 128, 128), 128)
            fwd = fwd_ref[...]
            prev = None
            for a in range(n_blk):
                cur = _dot_nt(fwd, g_vm[c, :, pl.ds(a * _BLK, _BLK)])
                if prev is None:
                    g_hat[a, spec, :] = cur
                else:
                    g_hat[a, 0:half, :] = cur[0:half] - prev[_BLK:_BLK + half]
                    g_hat[a, half:_BLK, :] = cur[half:_BLK] + prev[_BLK + half:]
                    g_hat[a, _BLK:_BLK + half, :] = cur[_BLK:_BLK + half] + prev[0:half]
                    g_hat[a, _BLK + half:2 * _BLK, :] = cur[_BLK + half:] - prev[half:_BLK]
                prev = cur
            kpad[8:8 + S, :] = k_vm[c].astype(f32)
            sh = shift_ref[:, cols].astype(f32)
            dsk = dskip_vm[:, cols]
            for a in range(n_blk):
                rows = pl.ds(a * _BLK, _BLK)
                acc = kpad[pl.ds(8 + a * _BLK, _BLK), :] * sh[0:1, :]
                for i in range(1, ks):
                    acc = acc + kpad[pl.ds(8 + a * _BLK - i, _BLK), :] * sh[i:i + 1, :]
                kv = acc * v_vm[c, rows, :].astype(f32)
                skip[rows, cols] = kv * dsk
                u_hat[a, spec, :] = _dot(fwd, kv.astype(bf16))

            def product_body(i, carry2):
                j = n_plain + 2 * c + i
                fetch_pair(j)
                n_rows = n_seg * _PRE
                pace = []
                for m in range(3):
                    total = None
                    for kt in range(n_ct):
                        kk = slice(kt * 128, (kt + 1) * 128)
                        t = _dot_nt(xsel[:, kk], stage[j % 2, m, :, kk])
                        pace += [t[q:q + 8, 0:128] for q in range(0, n_rows, 8)]
                        total = t if total is None else total + t
                    pre[j, :, m * PW:(m + 1) * PW] = total
                repack_pair(j)
                n_freq = _BLK // 2
                n_mac = (n_freq // 8) * n_blk * (n_blk + 1) // 2
                done = 0
                for r in range(0, n_freq, 8):
                    re = pl.ds(pl.multiple_of(i * n_freq + r, 8), 8)
                    im = pl.ds(pl.multiple_of(i * n_freq + r + _BLK, 8), 8)
                    for a0 in range(0, n_blk, 2):
                        yr, yi = {}, {}
                        for b in range(a0 + 2):
                            gr, gi = g_hat[b, re, :], g_hat[b, im, :]
                            if b % 2 == 0:
                                gr = jnp.where(i < 0, pace[done * len(pace) // n_mac], gr)
                            for a in range(max(b, a0), a0 + 2):
                                ur, ui = u_hat[a - b, re, :], u_hat[a - b, im, :]
                                tr, ti = gr * ur - gi * ui, gr * ui + gi * ur
                                yr[a] = yr[a] + tr if a in yr else tr
                                yi[a] = yi[a] + ti if a in yi else ti
                                done += 1
                        for a in yr:
                            y = jnp.concatenate([yr[a], yi[a]], axis=0).astype(bf16)
                            y_hat[a, re, cols] = pltpu.bitcast(y, u32)
                return carry2

            jax.lax.fori_loop(0, 2, product_body, 0)
            return carry

        jax.lax.fori_loop(0, n_ct, conv_body, 0)
        x_copy.wait()

        row = jax.lax.broadcasted_iota(jnp.int32, (L, 2 * L), 0)
        col = jax.lax.broadcasted_iota(jnp.int32, (L, 2 * L), 1)
        first = col < L
        visible = (row < M) | (row >= jnp.where(first, col, col - L))
        lane_first = jax.lax.broadcasted_iota(jnp.int32, (L, PW), 1) < Dh
        gw = gw_ref[...].astype(f32).reshape(1, D)

        def stack(t):
            zero = jnp.zeros_like(t)
            both = jnp.concatenate(
                [jnp.where(lane_first, t, zero), jnp.where(lane_first, zero, t)], axis=0)
            return both.astype(bf16)

        def step(blk, part, mem):
            s = blk * per_blk + part
            xs = x_vm[s].astype(f32)
            h = jnp.concatenate([mem, xs[0:seg - _PRE]], axis=0).astype(bf16)
            ahead = pl.ds(pl.multiple_of(s * _PRE, _PRE), _PRE)
            qkv, p, o = {}, {}, {}
            acc = None
            for op, j in _step_schedule(n_pair):
                if op == "P":
                    qkv[j] = jnp.concatenate(
                        [_dot(h, pltpu.bitcast(wqkv[j], bf16)), pre[j, ahead, :]], axis=0)
                elif op == "S":
                    sc = _dot_nt(qkv[j][:, 0:PW], stack(qkv[j][:, PW:2 * PW])) * scale
                    sc = jnp.where(visible, sc, -1e9)
                    m0 = jnp.max(jnp.where(first, sc, -jnp.inf), axis=-1, keepdims=True)
                    m1 = jnp.max(jnp.where(first, -jnp.inf, sc), axis=-1, keepdims=True)
                    e = jnp.exp(sc - jnp.where(first, m0, m1))
                    s0 = jnp.sum(jnp.where(first, e, 0.0), axis=-1, keepdims=True)
                    s1 = jnp.sum(jnp.where(first, 0.0, e), axis=-1, keepdims=True)
                    p[j] = e / jnp.where(first, s0, s1)
                elif op == "V":
                    o[j] = _dot(p[j], stack(qkv[j][:, 2 * PW:]))
                elif op == "O":
                    t = _dot(o[j], pltpu.bitcast(wo_vm[j], bf16))
                    acc = t if acc is None else acc + t
                else:
                    y = _dot(inv_ref[part * seg:(part + 1) * seg, :],
                             pltpu.bitcast(y_hat[blk], bf16))
            b = xs * (y + skip[pl.ds(pl.multiple_of(s * seg, seg), seg), :])
            gate = jax.nn.sigmoid(jnp.sum(xs * gw, axis=-1, keepdims=True))
            out_vm[s] = (gate * acc[M:] + (1.0 - gate) * b).astype(bf16)
            return acc[0:M]

        def steps(blk, mem):
            for part in range(per_blk):
                mem = step(blk, part, mem)
            segs = pl.ds(blk * per_blk, per_blk)
            pltpu.make_async_copy(out_vm.at[segs], out_hbm.at[segs], out_sem).start()
            return mem

        jax.lax.fori_loop(0, n_blk, steps, mem0_ref[...].astype(f32))
        pltpu.make_async_copy(out_vm, out_hbm, out_sem).wait()

    return kernel


def pallas_gated_mix__memory_aug_recurrent_mem_tr__ssm_conv_h3__prompt_kernel(
    A_x, A_mem0, A_Wq, A_Wk, A_Wv, A_Wo, A_seg_len, B_q, B_k, B_v,
    B_shift_k, B_ssm_k, B_ssm_D, gate_w,
):
    del B_q
    seg = int(A_seg_len)
    B, S, D = A_x.shape
    _, H, Dh = A_Wq.shape
    M = A_mem0.shape[1]
    ks = B_shift_k.shape[1]
    PW = 2 * Dh
    n_pair = H // 2
    n_blk = S // _BLK
    n_seg = S // seg
    assert B == 1 and H % 2 == 0 and PW % 128 == 0 and D % 128 == 0
    assert S % _BLK == 0 and _BLK % seg == 0 and seg % 16 == 0
    assert M % 8 == 0 and ks <= 8 and n_pair >= 2 * (D // 128) + 4
    f32, bf16, u32 = jnp.float32, jnp.bfloat16, jnp.uint32
    fwd, inv = _dft_matrices()

    def heads_major(w):
        return jnp.transpose(w, (1, 2, 0)).reshape(H * Dh, D)

    hbm = pl.BlockSpec(memory_space=pl.ANY)
    vmem = pl.BlockSpec(memory_space=pltpu.VMEM)
    out = pl.pallas_call(
        _make_kernel(S, D, H, Dh, M, seg, ks),
        out_shape=jax.ShapeDtypeStruct((n_seg, seg, D), A_x.dtype),
        in_specs=[hbm, vmem, hbm, hbm, hbm, hbm, hbm, hbm,
                  vmem, hbm, vmem, vmem, vmem, vmem],
        out_specs=hbm,
        scratch_shapes=[
            pltpu.VMEM((n_seg, seg, D), bf16),
            pltpu.VMEM((n_seg, _PRE, D), bf16),
            pltpu.VMEM((n_seg * _PRE, D), bf16),
            pltpu.VMEM((D // 128, S, 128), bf16),
            pltpu.VMEM((D // 128, S, 128), bf16),
            pltpu.VMEM((D // 128, 128, S), bf16),
            pltpu.VMEM((2, 4, PW, D), bf16),
            pltpu.VMEM((n_pair, D // 2, 3 * PW), u32),
            pltpu.VMEM((n_pair, PW // 2, D), u32),
            pltpu.VMEM((n_pair, n_seg * _PRE, 3 * PW), f32),
            pltpu.VMEM((1, D), f32),
            pltpu.VMEM((S + 8, 128), f32),
            pltpu.VMEM((n_blk, 2 * _BLK + 24, 128), f32),
            pltpu.VMEM((n_blk, 2 * _BLK + 40, 128), f32),
            pltpu.VMEM((n_blk, _BLK, D), u32),
            pltpu.VMEM((S, D), f32),
            pltpu.VMEM((n_seg, seg, D), bf16),
            pltpu.SemaphoreType.DMA((2,)),
            pltpu.SemaphoreType.DMA((D // 128,)),
            pltpu.SemaphoreType.DMA((2 * 4,)),
            pltpu.SemaphoreType.DMA(()),
        ],
        compiler_params=pltpu.CompilerParams(vmem_limit_bytes=120 * 1024 * 1024),
    )(
        A_x.reshape(n_seg, seg, D), A_mem0.reshape(M, D),
        heads_major(A_Wq), heads_major(A_Wk), heads_major(A_Wv),
        A_Wo.reshape(H * Dh, D), B_k.reshape(S, D), B_v.reshape(S, D),
        B_shift_k.T, B_ssm_k, B_ssm_D, gate_w,
        jnp.asarray(fwd, bf16), jnp.asarray(inv, bf16),
    )
    return out.reshape(B, S, D)
```

```python
import numpy as np

import jax
import jax.numpy as jnp
import jax.experimental.pallas as pl
import jax.experimental.pallas.tpu as pltpu

_BLK = 128
_PRE = 8
_ORDER, _LAG, _TAIL = "POVS", dict(S=1, V=3, O=9), "OOVSOOVOOOVOOF"


def _dft_matrices():
    f = np.concatenate([np.arange(0, _BLK, 2), np.arange(1, _BLK, 2)])
    t = np.arange(_BLK)
    ang = 2.0 * np.pi * (f[:, None] + 0.5) * t[None, :] / (2 * _BLK)
    fwd = np.concatenate([np.cos(ang), -np.sin(ang)], axis=0)
    inv = fwd.reshape(2, _BLK // 8, 8, _BLK).transpose(3, 1, 0, 2).reshape(_BLK, 2 * _BLK)
    inv = inv / _BLK
    return fwd.astype(np.float32), inv.astype(np.float32)


def _dot(a, b):
    return jax.lax.dot_general(
        a, b, (((1,), (0,)), ((), ())), preferred_element_type=jnp.float32)


def _dot_nt(a, b):
    return jax.lax.dot_general(
        a, b, (((1,), (1,)), ((), ())), preferred_element_type=jnp.float32)


def _step_schedule(n):
    lag = dict(P=0, **_LAG)
    done = dict.fromkeys("PSVOF", 0)
    sched = []

    def emit(op):
        if done[op] < n:
            sched.append((op, done[op]))
            done[op] += 1

    for j in range(n):
        for op in _ORDER:
            if j >= lag[op]:
                emit(op)
    for op in _TAIL:
        emit(op)
    assert all(done[op] == n for op in "PSVO") and done["F"] == 1
    return sched


def _make_kernel(S, D, H, Dh, M, seg, ks):
    L = M + seg
    n_seg = S // seg
    n_pair = H // 2
    PW = 2 * Dh
    n_blk = S // _BLK
    n_ct = D // 128
    n_plain = n_pair - 2 * n_ct
    half = _BLK // 2
    per_blk = _BLK // seg
    spec = slice(0, 2 * _BLK)
    scale = float(Dh) ** -0.5
    f32, bf16, u32 = jnp.float32, jnp.bfloat16, jnp.uint32

    def kernel(x_hbm, mem0_ref, wq_hbm, wk_hbm, wv_hbm, wo_hbm, k_hbm, v_hbm,
               shift_ref, g_hbm, dskip_ref, gw_ref, fwd_ref, inv_ref,
               out_hbm,
               x_vm, xs_vm, xsel, k_vm, v_vm, g_vm, stage, wqkv, wo_vm, pre,
               dskip_vm, kpad, u_hat, g_hat, y_hat, skip, out_vm,
               in_sem, tile_sem, w_sem, out_sem):
        xs_copy = pltpu.make_async_copy(
            x_hbm.at[:, pl.ds(seg - _PRE, _PRE), :], xs_vm, in_sem.at[0])
        x_copy = pltpu.make_async_copy(x_hbm, x_vm, in_sem.at[1])

        def tile_copies(c):
            cols = pl.ds(pl.multiple_of(c * 128, 128), 128)
            return [
                pltpu.make_async_copy(g_hbm.at[cols, :], g_vm.at[c], tile_sem.at[c]),
                pltpu.make_async_copy(k_hbm.at[:, cols], k_vm.at[c], tile_sem.at[c]),
                pltpu.make_async_copy(v_hbm.at[:, cols], v_vm.at[c], tile_sem.at[c]),
            ]

        def w_copies(j, slot):
            rows = pl.ds(pl.multiple_of(j * PW, PW), PW)
            return [
                pltpu.make_async_copy(
                    src.at[rows, :], stage.at[slot, m], w_sem.at[slot * 4 + m])
                for m, src in enumerate((wq_hbm, wk_hbm, wv_hbm, wo_hbm))]

        def tile_pairs(c):
            return [(n_plain + 2 * c + i, 2 + 2 * (c % 2) + i) for i in range(2)]

        def conv_copies(c):
            return tile_copies(c) + sum((w_copies(*js) for js in tile_pairs(c)), [])

        def repack_pair(j, slot):
            for m in range(3):
                wqkv[j, :, m * PW:(m + 1) * PW] = pltpu.bitcast(stage[slot, m].T, u32)
            wo_vm[j] = pltpu.bitcast(stage[slot, 3], u32)

        def project_ahead(j, slot, m):
            pre[j, :, m * PW:(m + 1) * PW] = _dot_nt(xsel[...], stage[slot, m])

        first_copies = w_copies(0, 0)
        xs_copy.start()
        first_copies[0].start()
        kpad[0:8, :] = jnp.zeros((8, 128), f32)
        dskip_vm[...] = dskip_ref[...].astype(f32).reshape(1, D)
        xs_copy.wait()
        first_copies[0].wait()
        for copy in first_copies[1:3]:
            copy.start()
        xsel[...] = xs_vm[...].astype(f32).reshape(n_seg * _PRE, D).astype(bf16)
        project_ahead(0, 0, 0)
        for copy in first_copies[1:3]:
            copy.wait()
        for copy in first_copies[3:] + w_copies(1, 1):
            copy.start()
        project_ahead(0, 0, 1)
        project_ahead(0, 0, 2)
        first_copies[3].wait()
        repack_pair(0, 0)

        def plain_body(j, carry):
            @pl.when(j + 1 < n_plain)
            def _():
                for copy in w_copies(j + 1, (j + 1) % 2):
                    copy.start()

            for i, early in enumerate(conv_copies(0)):
                @pl.when(j == min(1 + i // 2, n_plain - 1))
                def _():
                    early.start()

            for copy in w_copies(j, j % 2):
                copy.wait()
            for m in range(3):
                project_ahead(j, j % 2, m)
            repack_pair(j, j % 2)
            return carry

        jax.lax.fori_loop(1, n_plain, plain_body, 0)

        def conv_body(c, carry):
            @pl.when(c + 1 < n_ct)
            def _():
                for copy in conv_copies(c + 1):
                    copy.start()

            @pl.when(c + 1 == n_ct)
            def _():
                x_copy.start()

            for copy in conv_copies(c):
                copy.wait()
            cols = pl.ds(pl.multiple_of(c * 128, 128), 128)
            fwd = fwd_ref[...]
            prev = None
            for a in range(n_blk):
                cur = _dot_nt(fwd, g_vm[c, :, pl.ds(a * _BLK, _BLK)])
                if prev is None:
                    g_hat[a, spec, :] = cur
                else:
                    g_hat[a, 0:half, :] = cur[0:half] - prev[_BLK:_BLK + half]
                    g_hat[a, half:_BLK, :] = cur[half:_BLK] + prev[_BLK + half:]
                    g_hat[a, _BLK:_BLK + half, :] = cur[_BLK:_BLK + half] + prev[0:half]
                    g_hat[a, _BLK + half:2 * _BLK, :] = cur[_BLK + half:] - prev[half:_BLK]
                prev = cur
            kpad[8:8 + S, :] = k_vm[c].astype(f32)
            sh = shift_ref[:, cols].astype(f32)
            dsk = dskip_vm[:, cols]
            for a in range(n_blk):
                rows = pl.ds(a * _BLK, _BLK)
                acc = kpad[pl.ds(8 + a * _BLK, _BLK), :] * sh[0:1, :]
                for i in range(1, ks):
                    acc = acc + kpad[pl.ds(8 + a * _BLK - i, _BLK), :] * sh[i:i + 1, :]
                kv = acc * v_vm[c, rows, :].astype(f32)
                skip[rows, cols] = kv * dsk
                u_hat[a, spec, :] = _dot(fwd, kv.astype(bf16))

            n_rows = n_seg * _PRE
            pace = []
            for j, slot in tile_pairs(c):
                for m in range(3):
                    total = None
                    for kt in range(n_ct):
                        kk = slice(kt * 128, (kt + 1) * 128)
                        t = _dot_nt(xsel[:, kk], stage[slot, m, :, kk])
                        pace += [t[q:q + 8, 0:128] for q in range(0, n_rows, 8)]
                        total = t if total is None else total + t
                    pre[j, :, m * PW:(m + 1) * PW] = total
                repack_pair(j, slot)

            never = c < 0
            base = jnp.where(never, 8, 0)
            n_mac = (_BLK // 8) * n_blk * (n_blk + 1) // 2
            done = 0
            for r in range(0, _BLK, 8):
                re = pl.ds(pl.multiple_of(base + r, 8), 8)
                im = pl.ds(pl.multiple_of(base + r + _BLK, 8), 8)
                for a0 in range(0, n_blk, 2):
                    yr, yi = {}, {}
                    for b in range(a0 + 2):
                        gr, gi = g_hat[b, re, :], g_hat[b, im, :]
                        if b % 2 == 0:
                            gr = jnp.where(never, pace[done * len(pace) // n_mac], gr)
                        for a in range(max(b, a0), a0 + 2):
                            ur, ui = u_hat[a - b, re, :], u_hat[a - b, im, :]
                            tr, ti = gr * ur - gi * ui, gr * ui + gi * ur
                            yr[a] = yr[a] + tr if a in yr else tr
                            yi[a] = yi[a] + ti if a in yi else ti
                            done += 1
                    for a in yr:
                        y = jnp.concatenate([yr[a], yi[a]], axis=0).astype(bf16)
                        y_hat[a, r:r + 8, cols] = pltpu.bitcast(y, u32)
            return carry

        jax.lax.fori_loop(0, n_ct, conv_body, 0)
        x_copy.wait()

        row = jax.lax.broadcasted_iota(jnp.int32, (L, 2 * L), 0)
        col = jax.lax.broadcasted_iota(jnp.int32, (L, 2 * L), 1)
        first = col < L
        visible = (row < M) | (row >= jnp.where(first, col, col - L))
        lane_first = jax.lax.broadcasted_iota(jnp.int32, (L, PW), 1) < Dh
        gw = gw_ref[...].astype(f32).reshape(1, D)

        def stack(t):
            zero = jnp.zeros_like(t)
            both = jnp.concatenate(
                [jnp.where(lane_first, t, zero), jnp.where(lane_first, zero, t)], axis=0)
            return both.astype(bf16)

        def step(blk, part, mem):
            s = blk * per_blk + part
            xs = x_vm[s].astype(f32)
            h = jnp.concatenate([mem, xs[0:seg - _PRE]], axis=0).astype(bf16)
            ahead = pl.ds(pl.multiple_of(s * _PRE, _PRE), _PRE)
            qkv, p, o = {}, {}, {}
            acc = None
            for op, j in _step_schedule(n_pair):
                if op == "P":
                    qkv[j] = jnp.concatenate(
                        [_dot(h, pltpu.bitcast(wqkv[j], bf16)), pre[j, ahead, :]], axis=0)
                elif op == "S":
                    sc = _dot_nt(qkv[j][:, 0:PW], stack(qkv[j][:, PW:2 * PW])) * scale
                    sc = jnp.where(visible, sc, -1e9)
                    m0 = jnp.max(jnp.where(first, sc, -jnp.inf), axis=-1, keepdims=True)
                    m1 = jnp.max(jnp.where(first, -jnp.inf, sc), axis=-1, keepdims=True)
                    e = jnp.exp(sc - jnp.where(first, m0, m1))
                    s0 = jnp.sum(jnp.where(first, e, 0.0), axis=-1, keepdims=True)
                    s1 = jnp.sum(jnp.where(first, 0.0, e), axis=-1, keepdims=True)
                    p[j] = e / jnp.where(first, s0, s1)
                elif op == "V":
                    o[j] = _dot(p[j], stack(qkv[j][:, 2 * PW:]))
                elif op == "O":
                    t = _dot(o[j], pltpu.bitcast(wo_vm[j], bf16))
                    acc = t if acc is None else acc + t
                else:
                    y = _dot(inv_ref[part * seg:(part + 1) * seg, :],
                             pltpu.bitcast(y_hat[blk], bf16))
            b = xs * (y + skip[pl.ds(pl.multiple_of(s * seg, seg), seg), :])
            gate = jax.nn.sigmoid(jnp.sum(xs * gw, axis=-1, keepdims=True))
            out_vm[s] = (gate * acc[M:] + (1.0 - gate) * b).astype(bf16)
            return acc[0:M]

        def steps(blk, mem):
            for part in range(per_blk):
                mem = step(blk, part, mem)
            segs = pl.ds(blk * per_blk, per_blk)
            pltpu.make_async_copy(out_vm.at[segs], out_hbm.at[segs], out_sem).start()
            return mem

        jax.lax.fori_loop(0, n_blk, steps, mem0_ref[...].astype(f32))
        pltpu.make_async_copy(out_vm, out_hbm, out_sem).wait()

    return kernel


def pallas_gated_mix__memory_aug_recurrent_mem_tr__ssm_conv_h3__prompt_kernel(
    A_x, A_mem0, A_Wq, A_Wk, A_Wv, A_Wo, A_seg_len, B_q, B_k, B_v,
    B_shift_k, B_ssm_k, B_ssm_D, gate_w,
):
    del B_q
    seg = int(A_seg_len)
    B, S, D = A_x.shape
    _, H, Dh = A_Wq.shape
    M = A_mem0.shape[1]
    ks = B_shift_k.shape[1]
    PW = 2 * Dh
    n_pair = H // 2
    n_blk = S // _BLK
    n_seg = S // seg
    assert B == 1 and H % 2 == 0 and PW % 128 == 0 and D % 128 == 0
    assert S % _BLK == 0 and _BLK % seg == 0 and seg % 16 == 0
    assert M % 8 == 0 and ks <= 8 and n_pair >= 2 * (D // 128) + 2
    f32, bf16, u32 = jnp.float32, jnp.bfloat16, jnp.uint32
    fwd, inv = _dft_matrices()

    def heads_major(w):
        return jnp.transpose(w, (1, 2, 0)).reshape(H * Dh, D)

    hbm = pl.BlockSpec(memory_space=pl.ANY)
    vmem = pl.BlockSpec(memory_space=pltpu.VMEM)
    out = pl.pallas_call(
        _make_kernel(S, D, H, Dh, M, seg, ks),
        out_shape=jax.ShapeDtypeStruct((n_seg, seg, D), A_x.dtype),
        in_specs=[hbm, vmem, hbm, hbm, hbm, hbm, hbm, hbm,
                  vmem, hbm, vmem, vmem, vmem, vmem],
        out_specs=hbm,
        scratch_shapes=[
            pltpu.VMEM((n_seg, seg, D), bf16),
            pltpu.VMEM((n_seg, _PRE, D), bf16),
            pltpu.VMEM((n_seg * _PRE, D), bf16),
            pltpu.VMEM((D // 128, S, 128), bf16),
            pltpu.VMEM((D // 128, S, 128), bf16),
            pltpu.VMEM((D // 128, 128, S), bf16),
            pltpu.VMEM((6, 4, PW, D), bf16),
            pltpu.VMEM((n_pair, D // 2, 3 * PW), u32),
            pltpu.VMEM((n_pair, PW // 2, D), u32),
            pltpu.VMEM((n_pair, n_seg * _PRE, 3 * PW), f32),
            pltpu.VMEM((1, D), f32),
            pltpu.VMEM((S + 8, 128), f32),
            pltpu.VMEM((n_blk, 2 * _BLK + 8, 128), f32),
            pltpu.VMEM((n_blk, 2 * _BLK + 24, 128), f32),
            pltpu.VMEM((n_blk, _BLK, D), u32),
            pltpu.VMEM((S, D), f32),
            pltpu.VMEM((n_seg, seg, D), bf16),
            pltpu.SemaphoreType.DMA((2,)),
            pltpu.SemaphoreType.DMA((D // 128,)),
            pltpu.SemaphoreType.DMA((6 * 4,)),
            pltpu.SemaphoreType.DMA(()),
        ],
        compiler_params=pltpu.CompilerParams(vmem_limit_bytes=120 * 1024 * 1024),
    )(
        A_x.reshape(n_seg, seg, D), A_mem0.reshape(M, D),
        heads_major(A_Wq), heads_major(A_Wk), heads_major(A_Wv),
        A_Wo.reshape(H * Dh, D), B_k.reshape(S, D), B_v.reshape(S, D),
        B_shift_k.T, B_ssm_k, B_ssm_D, gate_w,
        jnp.asarray(fwd, bf16), jnp.asarray(inv, bf16),
    )
    return out.reshape(B, S, D)
```

```python
import numpy as np

import jax
import jax.numpy as jnp
import jax.experimental.pallas as pl
import jax.experimental.pallas.tpu as pltpu

_BLK = 128
_PRE = 8
_ORDER, _LAG, _TAIL = "POVS", dict(S=1, V=3, O=9), "OOVSOOVOOOVOOF"


def _dft_matrices():
    f = np.concatenate([np.arange(0, _BLK, 2), np.arange(1, _BLK, 2)])
    t = np.arange(_BLK)
    ang = 2.0 * np.pi * (f[:, None] + 0.5) * t[None, :] / (2 * _BLK)
    fwd = np.concatenate([np.cos(ang), -np.sin(ang)], axis=0)
    inv = fwd.reshape(2, _BLK // 8, 8, _BLK).transpose(3, 1, 0, 2).reshape(_BLK, 2 * _BLK)
    inv = inv / _BLK
    return fwd.astype(np.float32), inv.astype(np.float32)


def _dot(a, b):
    return jax.lax.dot_general(
        a, b, (((1,), (0,)), ((), ())), preferred_element_type=jnp.float32)


def _dot_nt(a, b):
    return jax.lax.dot_general(
        a, b, (((1,), (1,)), ((), ())), preferred_element_type=jnp.float32)


def _step_schedule(n):
    lag = dict(P=0, **_LAG)
    done = dict.fromkeys("PSVOF", 0)
    sched = []

    def emit(op):
        if done[op] < n:
            sched.append((op, done[op]))
            done[op] += 1

    for j in range(n):
        for op in _ORDER:
            if j >= lag[op]:
                emit(op)
    for op in _TAIL:
        emit(op)
    assert all(done[op] == n for op in "PSVO") and done["F"] == 1
    return sched


def _make_kernel(S, D, H, Dh, M, seg, ks):
    L = M + seg
    n_seg = S // seg
    n_pair = H // 2
    PW = 2 * Dh
    n_blk = S // _BLK
    n_ct = D // 128
    n_plain = n_pair - 2 * n_ct
    half = _BLK // 2
    per_blk = _BLK // seg
    spec = slice(0, 2 * _BLK)
    scale = float(Dh) ** -0.5
    f32, bf16, u32 = jnp.float32, jnp.bfloat16, jnp.uint32

    def kernel(x_hbm, mem0_ref, wq_hbm, wk_hbm, wv_hbm, wo_hbm, k_hbm, v_hbm,
               shift_ref, g_hbm, dskip_ref, gw_ref, fwd_ref, inv_ref,
               out_hbm,
               x_vm, xs_vm, xsel, k_vm, v_vm, g_vm, stage, wqkv, wo_vm, pre,
               dskip_vm, kpad, u_hat, g_hat, y_hat, skip, out_vm,
               in_sem, tile_sem, w_sem, out_sem):
        xs_copy = pltpu.make_async_copy(
            x_hbm.at[:, pl.ds(seg - _PRE, _PRE), :], xs_vm, in_sem.at[0])
        x_copy = pltpu.make_async_copy(x_hbm, x_vm, in_sem.at[1])

        def tile_copies(c):
            cols = pl.ds(pl.multiple_of(c * 128, 128), 128)
            return [
                pltpu.make_async_copy(g_hbm.at[cols, :], g_vm.at[c], tile_sem.at[c]),
                pltpu.make_async_copy(k_hbm.at[:, cols], k_vm.at[c], tile_sem.at[c]),
                pltpu.make_async_copy(v_hbm.at[:, cols], v_vm.at[c], tile_sem.at[c]),
            ]

        def w_copies(j, slot):
            rows = pl.ds(pl.multiple_of(j * PW, PW), PW)
            return [
                pltpu.make_async_copy(
                    src.at[rows, :], stage.at[slot, m], w_sem.at[slot * 4 + m])
                for m, src in enumerate((wq_hbm, wk_hbm, wv_hbm, wo_hbm))]

        def tile_pairs(c):
            return [(n_plain + 2 * c + i, 2 + 2 * (c % 2) + i) for i in range(2)]

        def conv_copies(c):
            return tile_copies(c) + sum((w_copies(*js) for js in tile_pairs(c)), [])

        def repack_pair(j, slot):
            for m in range(3):
                wqkv[j, :, m * PW:(m + 1) * PW] = pltpu.bitcast(stage[slot, m].T, u32)
            wo_vm[j] = pltpu.bitcast(stage[slot, 3], u32)

        def project_ahead(j, slot, m):
            pre[j, :, m * PW:(m + 1) * PW] = _dot_nt(xsel[...], stage[slot, m])

        first_copies = w_copies(0, 0)
        xs_copy.start()
        first_copies[0].start()
        kpad[0:8, :] = jnp.zeros((8, 128), f32)
        dskip_vm[...] = dskip_ref[...].astype(f32).reshape(1, D)
        xs_copy.wait()
        first_copies[0].wait()
        for copy in first_copies[1:3]:
            copy.start()
        xsel[...] = xs_vm[...].astype(f32).reshape(n_seg * _PRE, D).astype(bf16)
        project_ahead(0, 0, 0)
        for copy in first_copies[1:3]:
            copy.wait()
        for copy in first_copies[3:] + w_copies(1, 1):
            copy.start()
        project_ahead(0, 0, 1)
        project_ahead(0, 0, 2)
        first_copies[3].wait()
        repack_pair(0, 0)

        def plain_body(j, carry):
            @pl.when(j + 1 < n_plain)
            def _():
                for copy in w_copies(j + 1, (j + 1) % 2):
                    copy.start()

            for i, early in enumerate(conv_copies(0)):
                @pl.when(j == min(1 + i // 2, n_plain - 1))
                def _():
                    early.start()

            for copy in w_copies(j, j % 2):
                copy.wait()
            for m in range(3):
                project_ahead(j, j % 2, m)
            repack_pair(j, j % 2)
            return carry

        jax.lax.fori_loop(1, n_plain, plain_body, 0)

        def conv_body(c, carry):
            @pl.when(c + 1 < n_ct)
            def _():
                for copy in conv_copies(c + 1):
                    copy.start()

            @pl.when(c + 1 == n_ct)
            def _():
                x_copy.start()

            for copy in conv_copies(c):
                copy.wait()
            cols = pl.ds(pl.multiple_of(c * 128, 128), 128)
            fwd = fwd_ref[...]
            prev = None
            for a in range(n_blk):
                cur = _dot_nt(fwd, g_vm[c, :, pl.ds(a * _BLK, _BLK)])
                if prev is None:
                    g_hat[a, spec, :] = cur
                else:
                    g_hat[a, 0:half, :] = cur[0:half] - prev[_BLK:_BLK + half]
                    g_hat[a, half:_BLK, :] = cur[half:_BLK] + prev[_BLK + half:]
                    g_hat[a, _BLK:_BLK + half, :] = cur[_BLK:_BLK + half] + prev[0:half]
                    g_hat[a, _BLK + half:2 * _BLK, :] = cur[_BLK + half:] - prev[half:_BLK]
                prev = cur
            kpad[8:8 + S, :] = k_vm[c].astype(f32)
            sh = shift_ref[:, cols].astype(f32)
            dsk = dskip_vm[:, cols]
            for a in range(n_blk):
                rows = pl.ds(a * _BLK, _BLK)
                acc = kpad[pl.ds(8 + a * _BLK, _BLK), :] * sh[0:1, :]
                for i in range(1, ks):
                    acc = acc + kpad[pl.ds(8 + a * _BLK - i, _BLK), :] * sh[i:i + 1, :]
                kv = acc * v_vm[c, rows, :].astype(f32)
                skip[rows, cols] = kv * dsk
                u_hat[a, spec, :] = _dot(fwd, kv.astype(bf16))

            n_rows = n_seg * _PRE
            pace = []
            for j, slot in tile_pairs(c):
                for m in range(3):
                    total = None
                    for kt in range(n_ct):
                        kk = slice(kt * 128, (kt + 1) * 128)
                        t = _dot_nt(xsel[:, kk], stage[slot, m, :, kk])
                        pace += [t[q:q + 8, 0:128] for q in range(0, n_rows, 8)]
                        total = t if total is None else total + t
                    pre[j, :, m * PW:(m + 1) * PW] = total
                repack_pair(j, slot)

            never = c < 0
            base = jnp.where(never, 8, 0)
            n_mac = (_BLK // 8) * n_blk * (n_blk + 1) // 2
            done = 0
            for r in range(0, _BLK, 8):
                re = pl.ds(pl.multiple_of(base + r, 8), 8)
                im = pl.ds(pl.multiple_of(base + r + _BLK, 8), 8)
                ur, ui, gr, gi = (
                    [ref[a, rows, :] for a in range(n_blk)]
                    for ref, rows in ((u_hat, re), (u_hat, im), (g_hat, re), (g_hat, im)))
                for a0 in range(0, n_blk, 2):
                    yr, yi = {}, {}
                    for b in range(a0 + 2):
                        gre = gr[b]
                        if b % 2 == 0:
                            gre = jnp.where(never, pace[done * len(pace) // n_mac], gre)
                        for a in range(max(b, a0), a0 + 2):
                            tr = gre * ur[a - b] - gi[b] * ui[a - b]
                            ti = gre * ui[a - b] + gi[b] * ur[a - b]
                            yr[a] = yr[a] + tr if a in yr else tr
                            yi[a] = yi[a] + ti if a in yi else ti
                            done += 1
                    for a in yr:
                        y = jnp.concatenate([yr[a], yi[a]], axis=0).astype(bf16)
                        y_hat[a, r:r + 8, cols] = pltpu.bitcast(y, u32)
            return carry

        jax.lax.fori_loop(0, n_ct, conv_body, 0)
        x_copy.wait()

        row = jax.lax.broadcasted_iota(jnp.int32, (L, 2 * L), 0)
        col = jax.lax.broadcasted_iota(jnp.int32, (L, 2 * L), 1)
        first = col < L
        visible = (row < M) | (row >= jnp.where(first, col, col - L))
        lane_first = jax.lax.broadcasted_iota(jnp.int32, (L, PW), 1) < Dh
        gw = gw_ref[...].astype(f32).reshape(1, D)

        def stack(t):
            zero = jnp.zeros_like(t)
            both = jnp.concatenate(
                [jnp.where(lane_first, t, zero), jnp.where(lane_first, zero, t)], axis=0)
            return both.astype(bf16)

        def step(blk, part, mem):
            s = blk * per_blk + part
            xs = x_vm[s].astype(f32)
            h = jnp.concatenate([mem, xs[0:seg - _PRE]], axis=0).astype(bf16)
            ahead = pl.ds(pl.multiple_of(s * _PRE, _PRE), _PRE)
            qkv, p, o = {}, {}, {}
            acc = None
            for op, j in _step_schedule(n_pair):
                if op == "P":
                    qkv[j] = jnp.concatenate(
                        [_dot(h, pltpu.bitcast(wqkv[j], bf16)), pre[j, ahead, :]], axis=0)
                elif op == "S":
                    sc = _dot_nt(qkv[j][:, 0:PW], stack(qkv[j][:, PW:2 * PW])) * scale
                    sc = jnp.where(visible, sc, -1e9)
                    m0 = jnp.max(jnp.where(first, sc, -jnp.inf), axis=-1, keepdims=True)
                    m1 = jnp.max(jnp.where(first, -jnp.inf, sc), axis=-1, keepdims=True)
                    e = jnp.exp(sc - jnp.where(first, m0, m1))
                    s0 = jnp.sum(jnp.where(first, e, 0.0), axis=-1, keepdims=True)
                    s1 = jnp.sum(jnp.where(first, 0.0, e), axis=-1, keepdims=True)
                    p[j] = e / jnp.where(first, s0, s1)
                elif op == "V":
                    o[j] = _dot(p[j], stack(qkv[j][:, 2 * PW:]))
                elif op == "O":
                    t = _dot(o[j], pltpu.bitcast(wo_vm[j], bf16))
                    acc = t if acc is None else acc + t
                else:
                    y = _dot(inv_ref[part * seg:(part + 1) * seg, :],
                             pltpu.bitcast(y_hat[blk], bf16))
            conv = xs * (y + skip[pl.ds(pl.multiple_of(s * seg, seg), seg), :])
            gate = jax.nn.sigmoid(jnp.sum(xs * gw, axis=-1, keepdims=True))
            out_vm[s] = (gate * acc[M:] + (1.0 - gate) * conv).astype(bf16)
            return acc[0:M]

        def steps(blk, mem):
            for part in range(per_blk):
                mem = step(blk, part, mem)
            segs = pl.ds(blk * per_blk, per_blk)
            pltpu.make_async_copy(out_vm.at[segs], out_hbm.at[segs], out_sem).start()
            return mem

        jax.lax.fori_loop(0, n_blk, steps, mem0_ref[...].astype(f32))
        pltpu.make_async_copy(out_vm, out_hbm, out_sem).wait()

    return kernel


def pallas_gated_mix__memory_aug_recurrent_mem_tr__ssm_conv_h3__prompt_kernel(
    A_x, A_mem0, A_Wq, A_Wk, A_Wv, A_Wo, A_seg_len, B_q, B_k, B_v,
    B_shift_k, B_ssm_k, B_ssm_D, gate_w,
):
    del B_q
    seg = int(A_seg_len)
    B, S, D = A_x.shape
    _, H, Dh = A_Wq.shape
    M = A_mem0.shape[1]
    ks = B_shift_k.shape[1]
    PW = 2 * Dh
    n_pair = H // 2
    n_blk = S // _BLK
    n_seg = S // seg
    assert B == 1 and H % 2 == 0 and PW % 128 == 0 and D % 128 == 0
    assert S % _BLK == 0 and _BLK % seg == 0 and seg % 16 == 0
    assert M % 8 == 0 and ks <= 8 and n_pair >= 2 * (D // 128) + 2
    f32, bf16, u32 = jnp.float32, jnp.bfloat16, jnp.uint32
    fwd, inv = _dft_matrices()

    def heads_major(w):
        return jnp.transpose(w, (1, 2, 0)).reshape(H * Dh, D)

    hbm = pl.BlockSpec(memory_space=pl.ANY)
    vmem = pl.BlockSpec(memory_space=pltpu.VMEM)
    out = pl.pallas_call(
        _make_kernel(S, D, H, Dh, M, seg, ks),
        out_shape=jax.ShapeDtypeStruct((n_seg, seg, D), A_x.dtype),
        in_specs=[hbm, vmem, hbm, hbm, hbm, hbm, hbm, hbm,
                  vmem, hbm, vmem, vmem, vmem, vmem],
        out_specs=hbm,
        scratch_shapes=[
            pltpu.VMEM((n_seg, seg, D), bf16),
            pltpu.VMEM((n_seg, _PRE, D), bf16),
            pltpu.VMEM((n_seg * _PRE, D), bf16),
            pltpu.VMEM((D // 128, S, 128), bf16),
            pltpu.VMEM((D // 128, S, 128), bf16),
            pltpu.VMEM((D // 128, 128, S), bf16),
            pltpu.VMEM((6, 4, PW, D), bf16),
            pltpu.VMEM((n_pair, D // 2, 3 * PW), u32),
            pltpu.VMEM((n_pair, PW // 2, D), u32),
            pltpu.VMEM((n_pair, n_seg * _PRE, 3 * PW), f32),
            pltpu.VMEM((1, D), f32),
            pltpu.VMEM((S + 8, 128), f32),
            pltpu.VMEM((n_blk, 2 * _BLK + 8, 128), f32),
            pltpu.VMEM((n_blk, 2 * _BLK + 24, 128), f32),
            pltpu.VMEM((n_blk, _BLK, D), u32),
            pltpu.VMEM((S, D), f32),
            pltpu.VMEM((n_seg, seg, D), bf16),
            pltpu.SemaphoreType.DMA((2,)),
            pltpu.SemaphoreType.DMA((D // 128,)),
            pltpu.SemaphoreType.DMA((6 * 4,)),
            pltpu.SemaphoreType.DMA(()),
        ],
        compiler_params=pltpu.CompilerParams(vmem_limit_bytes=120 * 1024 * 1024),
    )(
        A_x.reshape(n_seg, seg, D), A_mem0.reshape(M, D),
        heads_major(A_Wq), heads_major(A_Wk), heads_major(A_Wv),
        A_Wo.reshape(H * Dh, D), B_k.reshape(S, D), B_v.reshape(S, D),
        B_shift_k.T, B_ssm_k, B_ssm_D, gate_w,
        jnp.asarray(fwd, bf16), jnp.asarray(inv, bf16),
    )
    return out.reshape(B, S, D)
```
